```python
import jax
import jax.numpy as jnp

def _softmax(x, axis=-1):
    return jax.nn.softmax(x, axis=axis)

def _gelu(x):
    return jax.nn.gelu(x, approximate=True)

def _silu(x):
    return jax.nn.silu(x)

def _sigmoid(x):
    return jax.nn.sigmoid(x)

def _layernorm(x, axis=-1, eps=1e-05):
    m = jnp.mean(x, axis=axis, keepdims=True)
    v = jnp.var(x, axis=axis, keepdims=True)
    return (x - m) / jnp.sqrt(v + eps)

def _scatter_add(tgt, idx, src, axis=0):
    return tgt.at[idx].add(src)

def _segment_sum(src, seg, n):
    return jax.ops.segment_sum(src, seg, n)

class _Rng:

    def __init__(self, key):
        self._k = key

    def _next(self):
        self._k, sub = jax.random.split(self._k)
        return sub

    def normal(self, shape):
        return jax.random.normal(self._next(), shape, dtype=jnp.bfloat16)

    def randint(self, lo, hi, shape):
        return jax.random.randint(self._next(), shape, lo, hi, dtype=jnp.int32)

    def uniform(self, shape, lo=0.0, hi=1.0):
        return jax.random.uniform(self._next(), shape, jnp.bfloat16, lo, hi)

    def permutation(self, n):
        return jax.random.permutation(self._next(), n)
kernel_name = 'interleave_layers__memory_aug_infini_attn__mixer_s_mlp__prompt'

def setup_inputs():
    _rng = _Rng(jax.random.key(int.from_bytes(__import__("os").urandom(4), "little")))
    _w = lambda a: (lambda t: t.astype(jnp.bfloat16) if jnp.issubdtype(t.dtype, jnp.floating) else t)(jnp.asarray(a))

    def _A_setup():
        B, S, D, H = (1, 2048, 1024, 32)
        N = 4
        L = max(1, S // N)
        sc = D ** (-0.5)
        return {'x': _w((lambda *s: _rng.normal(s) * 0.05)(B, N * L, D)), 'wq': _w((lambda *s: _rng.normal(s) * 0.05)(D, D) * sc), 'wk': _w((lambda *s: _rng.normal(s) * 0.05)(D, D) * sc), 'wv': _w((lambda *s: _rng.normal(s) * 0.05)(D, D) * sc), 'wo': _w((lambda *s: _rng.normal(s) * 0.05)(D, D) * sc), 'beta': _w((lambda *s: _rng.normal(s) * 0.05)(H))}
    _A_in = _A_setup()

    def _B_setup():
        B, S, D, F = (1, 2048, 1024, 3584)
        return {'x': _w((lambda *s: _rng.normal(s) * 0.05)(B, S, D)), 'w1': _w((lambda *s: _rng.normal(s) * 0.05)(D, D) * D ** (-0.5)), 'w2': _w((lambda *s: _rng.normal(s) * 0.05)(D, D) * D ** (-0.5)), 'w3': _w((lambda *s: _rng.normal(s) * 0.05)(D, F) * D ** (-0.5)), 'w4': _w((lambda *s: _rng.normal(s) * 0.05)(F, D) * F ** (-0.5))}
    _B_in = _B_setup()
    return {'A_x': _A_in['x'], 'A_wq': _A_in['wq'], 'A_wk': _A_in['wk'], 'A_wv': _A_in['wv'], 'A_wo': _A_in['wo'], 'A_beta': _A_in['beta'], 'B_x': _B_in['x'], 'B_w1': _B_in['w1'], 'B_w2': _B_in['w2'], 'B_w3': _B_in['w3'], 'B_w4': _B_in['w4']}

def reference(A_x, A_wq, A_wk, A_wv, A_wo, A_beta, B_x, B_w1, B_w2, B_w3, B_w4):

    def _A_ref(x, wq, wk, wv, wo, beta):
        B, S, D = x.shape
        H = 32
        Dh = D // H
        N = 4
        L = S // N
        q = (lambda x, *d: x.transpose(*d))((x @ wq).reshape(B, S, H, Dh), 0, 2, 1, 3).reshape(B, H, N, L, Dh)
        k = (lambda x, *d: x.transpose(*d))((x @ wk).reshape(B, S, H, Dh), 0, 2, 1, 3).reshape(B, H, N, L, Dh)
        v = (lambda x, *d: x.transpose(*d))((x @ wv).reshape(B, S, H, Dh), 0, 2, 1, 3).reshape(B, H, N, L, Dh)
        phi = lambda t: jnp.where(t > 0, t + 1.0, jnp.exp(t))
        scale = Dh ** (-0.5)
        ar = jnp.arange(L)
        mask = (lambda x, dt: x.astype(dt))(ar[:, None] < ar[None, :], x.dtype) * -1000000000.0
        g = _sigmoid(beta).reshape(1, H, 1, 1)
        M = jnp.einsum('bhd,bhe->bhde', q[:, :, 0, 0, :] * 0.0, q[:, :, 0, 0, :] * 0.0)
        z = q[:, :, 0, 0, :] * 0.0
        outs = []
        for s in range(N):
            qs, ks, vs = (q[:, :, s].copy(), k[:, :, s].copy(), v[:, :, s].copy())
            logits = jnp.einsum('bhqd,bhkd->bhqk', qs, ks) * scale + mask
            p = _softmax(logits, axis=-1)
            a_dot = jnp.einsum('bhqk,bhkd->bhqd', p, vs)
            pq = phi(qs)
            num = jnp.einsum('bhld,bhde->bhle', pq, M)
            den = jnp.einsum('bhld,bhd->bhl', pq, z)[..., None] + 1e-06
            a_mem = num / den
            o = g * a_mem + (1.0 - g) * a_dot
            outs.append(o)
            pk = phi(ks)
            M = M + jnp.einsum('bhld,bhle->bhde', pk, vs)
            z = z + jnp.einsum('bhld->bhd', pk)
        o = (lambda x, *d: x.transpose(*d))(jnp.stack(outs, 2).reshape(B, H, S, Dh), 0, 2, 1, 3).reshape(B, S, D)
        return o @ wo

    def _B_ref(x, w1, w2, w3, w4):
        B, S, D = x.shape
        h = _gelu(_layernorm(x, axis=-1) @ w1)
        c = D // 4
        g0 = jnp.pad(h[:, :, 0 * c:1 * c], ((0, 0), (1, 0), (0, 0)))[:, :S, :]
        g1 = jnp.pad(h[:, :, 1 * c:2 * c], ((0, 0), (0, 1), (0, 0)))[:, 1:, :]
        g2 = jnp.pad(h[:, :, 2 * c:3 * c], ((0, 0), (2, 0), (0, 0)))[:, :S, :]
        g3 = jnp.pad(h[:, :, 3 * c:], ((0, 0), (0, 2), (0, 0)))[:, 2:, :]
        hs = jnp.concatenate([g0, g1, g2, g3], axis=-1) @ w2
        x1 = x + hs
        h2 = _gelu(_layernorm(x1, axis=-1) @ w3) @ w4
        return x1 + h2
    x = A_x
    x = x + _A_ref(_layernorm(x, axis=-1), A_wq, A_wk, A_wv, A_wo, A_beta)
    x = x + _B_ref(_layernorm(x, axis=-1), B_w1, B_w2, B_w3, B_w4)
    x = x + _A_ref(_layernorm(x, axis=-1), A_wq, A_wk, A_wv, A_wo, A_beta)
    x = x + _B_ref(_layernorm(x, axis=-1), B_w1, B_w2, B_w3, B_w4)
    return x
```

```python
import math

import jax
import jax.numpy as jnp
from jax import lax
import jax.experimental.pallas as pl
import jax.experimental.pallas.tpu as pltpu

f32 = jnp.float32
bf16 = jnp.bfloat16

S = 2048
D = 1024
F = 3584
H = 32
DH = 32
L = 512
NSEG = S // L
NG = D // 128
TB = 256
FC = 512
HALO = 8
MZR = 144
EPS = 1e-5
NEG = -1e30
QSCALE = (DH ** -0.5) * math.log2(math.e)
GELU_C0 = math.sqrt(2.0 / math.pi)
GELU_C1 = GELU_C0 * 0.044715
ATT_LAG = 2


def _dot(a, b):
    return jnp.dot(a, b, preferred_element_type=f32)


def _dot_nt(a, b):
    return lax.dot_general(a, b, (((1,), (1,)), ((), ())), preferred_element_type=f32)


def _ln(x):
    m = jnp.mean(x, axis=-1, keepdims=True)
    xc = x - m
    v = jnp.mean(xc * xc, axis=-1, keepdims=True)
    return xc * lax.rsqrt(v + EPS)


def _gelu(x):
    t = jnp.tanh(x * (GELU_C0 + GELU_C1 * (x * x)))
    hx = 0.5 * x
    return hx + hx * t


def _phi(t):
    return jnp.where(t > 0, t + 1.0, jnp.exp(t))


def _fold(x, op):
    parts = [x[8 * i:8 * i + 8] for i in range(x.shape[0] // 8)]
    while len(parts) > 1:
        parts = [op(parts[i], parts[i + 1]) for i in range(0, len(parts), 2)]
    return parts[0]


def _attention(k_ref, qt_ref, pqt_ref, vt_ref, mz_ref, gate_ref, mask_ref, o_ref):
    steps = [(g, j, t) for g in range(NG) for j in range(4) for t in range(j + 1)]
    scores, run, mem, outs = {}, {}, {}, {}

    def do_qk(n):
        g, j, t = steps[n]
        if j == 0:
            mem[g] = _dot(mz_ref[g].astype(bf16), pqt_ref[128 * g:128 * g + 128, :])
        cols = []
        for h in range(4):
            r0 = 128 * g + 32 * h
            parts = []
            if h > 0:
                parts.append(jnp.zeros((32 * h, 128), bf16))
            parts.append(qt_ref[r0:r0 + 32, 128 * j:128 * j + 128])
            if h < 3:
                parts.append(jnp.zeros((96 - 32 * h, 128), bf16))
            cols.append(jnp.concatenate(parts, axis=0))
        w = jnp.concatenate(cols, axis=1)
        scores[n] = _dot(k_ref[128 * t:128 * t + 128, 128 * g:128 * g + 128], w)

    def do_sm(n):
        g, j, t = steps[n]
        st = scores.pop(n)
        cur = []
        for h in range(4):
            s = st[:, 128 * h:128 * h + 128]
            if t == j:
                s = s + mask_ref[...]
            m = jnp.max(_fold(s, jnp.maximum), axis=0, keepdims=True)
            if t > 0:
                m = jnp.maximum(m, run[h][0])
            cur.append((s, m))
        res = []
        for h in range(4):
            s, m = cur[h]
            r0 = 128 * g + 32 * h
            p = jnp.exp2(s - m)
            sm = _fold(p, jnp.add)
            o = _dot(vt_ref[r0:r0 + 32, 128 * t:128 * t + 128], p.astype(bf16))
            res.append((m, o, sm))
        for h in range(4):
            m, o, sm = res[h]
            if t > 0:
                a = jnp.exp2(run[h][0] - m)
                o = run[h][1] * a + o
                sm = run[h][2] * a + sm
            run[h] = (m, o, sm)
            if t == j:
                gate = gate_ref[4 * g + h:4 * g + h + 1, :]
                l = jnp.sum(sm, axis=0, keepdims=True)
                r = mem[g][:, 128 * j:128 * j + 128]
                den = r[128 + h:129 + h] + 1e-6
                outs[h] = r[32 * h:32 * h + 32] * (gate / den) + o * ((1.0 - gate) / l)
        if t == j:
            ot = jnp.concatenate([outs[h] for h in range(4)], axis=0)
            o_ref[128 * j:128 * j + 128, 128 * g:128 * g + 128] = ot.T.astype(bf16)

    n_steps = len(steps)
    for n in range(n_steps + ATT_LAG):
        if n < n_steps:
            do_qk(n)
        if n >= ATT_LAG:
            do_sm(n - ATT_LAG)


def _kernel(x_hbm, wq_hbm, wk_hbm, wv_hbm, wo_hbm, beta_hbm, w1_hbm, w2_hbm, w3_hbm, w4_hbm,
            out_hbm,
            xio, wq_s, wv_s, wk_v, wqvt, wo_v, w1_v, w2_v, w3_v, w4_v, beta_v,
            x_ref, y_ref, xn_ref, h_ref,
            k_ref, pk_ref, qt_ref, pqt_ref, vt_ref, o_ref,
            mz_ref, mzmask_ref, mask_ref, gate_ref,
            sem_in, sem_out):
    def cp(src, dst, i):
        return pltpu.make_async_copy(src, dst, sem_in.at[i])

    x_cp = [cp(x_hbm.at[pl.ds(L * s, L)], xio.at[pl.ds(L * s, L)], s) for s in range(NSEG)]
    wq_cp = cp(wq_hbm, wq_s, 4)
    wv_cp = cp(wv_hbm, wv_s, 5)
    wk_cp = cp(wk_hbm, wk_v, 6)
    beta_cp = cp(beta_hbm, beta_v, 7)
    wo_cp = cp(wo_hbm, wo_v, 8)
    w1_cp = cp(w1_hbm, w1_v, 9)
    w2_cp = cp(w2_hbm, w2_v, 10)
    w3_cp = cp(w3_hbm, w3_v, 11)
    w4_cp = cp(w4_hbm, w4_v, 12)

    def out_cp(t):
        r0 = pl.multiple_of(t * TB, TB)
        return pltpu.make_async_copy(xio.at[pl.ds(r0, TB)], out_hbm.at[pl.ds(r0, TB)], sem_out.at[t])

    for c in [beta_cp, wq_cp, wv_cp] + x_cp + [wk_cp]:
        c.start()

    kk = lax.broadcasted_iota(jnp.int32, (128, 128), 0)
    qq = lax.broadcasted_iota(jnp.int32, (128, 128), 1)
    mask_ref[...] = jnp.where(kk <= qq, 0.0, NEG).astype(f32)
    rr = lax.broadcasted_iota(jnp.int32, (MZR, 128), 0)
    cc = lax.broadcasted_iota(jnp.int32, (MZR, 128), 1) // DH
    row_head = jnp.where(rr < 128, rr // DH, rr - 128)
    mzmask_ref[...] = jnp.where(row_head == cc, 1.0, 0.0).astype(f32)
    h_ref[0:HALO, :] = jnp.zeros((HALO, D), f32)
    h_ref[HALO + S:HALO + S + HALO, :] = jnp.zeros((HALO, D), f32)

    beta_cp.wait()
    eye = (lax.broadcasted_iota(jnp.int32, (H, H), 0) == lax.broadcasted_iota(jnp.int32, (H, H), 1))
    beta_rows = jnp.broadcast_to(beta_v[...].astype(f32), (H, H))
    beta_col = jnp.sum(jnp.where(eye, beta_rows, 0.0), axis=1, keepdims=True)
    gate_ref[...] = jnp.broadcast_to(jax.nn.sigmoid(beta_col), (H, 128))

    wq_cp.wait()
    wqvt[0:D, :] = wq_s[...].T
    wv_cp.wait()
    wqvt[D:2 * D, :] = wv_s[...].T

    for s in range(NSEG):
        x_cp[s].wait()

    def ln_in(s, c):
        r0 = pl.multiple_of(s * TB, TB)
        xv = xio[pl.ds(r0, TB), :].astype(f32)
        x_ref[pl.ds(r0, TB), :] = xv
        xn_ref[pl.ds(r0, TB), :] = _ln(xv).astype(bf16)
        return c

    lax.fori_loop(0, S // TB, ln_in, 0)
    wk_cp.wait()
    for c in [wo_cp, w1_cp, w2_cp, w3_cp, w4_cp]:
        c.start()

    def seg_body(layer, s):
        r0 = pl.multiple_of(s * L, L)
        xn = xn_ref[pl.ds(r0, L), :]
        for c in range(2):
            cs = slice(512 * c, 512 * c + 512)
            kf = _dot(xn, wk_v[:, cs])
            k_ref[:, cs] = kf.astype(bf16)
            pk_ref[:, cs] = _phi(kf).astype(bf16)
        for c in range(2):
            rs = slice(512 * c, 512 * c + 512)
            qf = _dot_nt(wqvt[rs, :], xn)
            qt_ref[rs, :] = (qf * QSCALE).astype(bf16)
            pqt_ref[rs, :] = _phi(qf).astype(bf16)
        for c in range(2):
            rs = slice(512 * c, 512 * c + 512)
            vt_ref[rs, :] = _dot_nt(wqvt[D + 512 * c:D + 512 * c + 512, :], xn).astype(bf16)

        _attention(k_ref, qt_ref, pqt_ref, vt_ref, mz_ref, gate_ref, mask_ref, o_ref)

        ones = jnp.ones((MZR - 128, L), bf16)
        for g in range(NG):
            lhs = jnp.concatenate([vt_ref[128 * g:128 * g + 128, :], ones], axis=0)
            u = _dot(lhs, pk_ref[:, 128 * g:128 * g + 128])
            mz_ref[g] = mz_ref[g] + u * mzmask_ref[...]

        @pl.when(jnp.logical_and(layer == 0, s == 0))
        def _():
            wo_cp.wait()
            w1_cp.wait()

        half = L // 2
        yn = []
        for a in range(2):
            rows = pl.ds(pl.multiple_of(r0 + half * a, half), half)
            xv = x_ref[rows, :] + _dot(o_ref[half * a:half * a + half, :], wo_v[...])
            x_ref[rows, :] = xv
            y = _ln(xv)
            y_ref[rows, :] = y
            yn.append(_ln(y).astype(bf16))
        for a in range(2):
            rows = pl.ds(pl.multiple_of(r0 + half * a + HALO, 8), half)
            h_ref[rows, :] = _gelu(_dot(yn[a], w1_v[...]))

    def mix_body(layer, t):
        r0 = pl.multiple_of(t * TB, TB)
        half = TB // 2
        c4 = D // 4
        x1n, xr = [], []
        for a in range(2):
            ra = pl.multiple_of(r0 + half * a, half)
            win = h_ref[pl.ds(ra, half + 2 * HALO), :]
            hs_in = jnp.concatenate([
                win[HALO - 1:HALO - 1 + half, 0 * c4:1 * c4],
                win[HALO + 1:HALO + 1 + half, 1 * c4:2 * c4],
                win[HALO - 2:HALO - 2 + half, 2 * c4:3 * c4],
                win[HALO + 2:HALO + 2 + half, 3 * c4:4 * c4]], axis=1).astype(bf16)
            x1 = y_ref[pl.ds(ra, half), :] + _dot(hs_in, w2_v[...])
            xr.append(x_ref[pl.ds(ra, half), :] + x1)
            x1n.append(_ln(x1).astype(bf16))
        nch = F // FC
        x1n_full = jnp.concatenate(x1n, axis=0)

        def up(c):
            w = w3_v[:, FC * c:FC * c + FC]
            if c == 0:
                return jnp.concatenate([_gelu(_dot(x1n[a], w)) for a in range(2)], axis=0).astype(bf16)
            return _gelu(_dot(x1n_full, w)).astype(bf16)

        acc = jnp.concatenate(xr, axis=0)
        hcur = up(0)
        for c in range(nch):
            hnext = up(c + 1) if c + 1 < nch else None
            w = w4_v[FC * c:FC * c + FC, :]
            if c + 1 < nch:
                acc = acc + _dot(hcur, w)
            else:
                for a in range(2):
                    ra = pl.multiple_of(r0 + half * a, half)
                    xv = acc[half * a:half * a + half] + _dot(hcur[half * a:half * a + half], w)
                    x_ref[pl.ds(ra, half), :] = xv
                    xn_ref[pl.ds(ra, half), :] = _ln(xv).astype(bf16)
                    xio[pl.ds(ra, half), :] = xv.astype(bf16)
            hcur = hnext

        @pl.when(layer == 1)
        def _():
            out_cp(t).start()

    def layer_body(layer, carry):
        mz_ref[...] = jnp.zeros(mz_ref.shape, f32)

        def sb(s, c):
            seg_body(layer, s)
            return c

        lax.fori_loop(0, NSEG, sb, 0)

        @pl.when(layer == 0)
        def _():
            w2_cp.wait()
            w3_cp.wait()
            w4_cp.wait()

        def mb(t, c):
            mix_body(layer, t)
            return c

        lax.fori_loop(0, S // TB, mb, 0)
        return carry

    lax.fori_loop(0, 2, layer_body, 0)
    for t in range(S // TB):
        out_cp(t).wait()


@jax.jit
def pallas_interleave_layers__memory_aug_infini_attn__mixer_s_mlp__prompt_kernel(
    A_x: jax.Array,
    A_wq: jax.Array,
    A_wk: jax.Array,
    A_wv: jax.Array,
    A_wo: jax.Array,
    A_beta: jax.Array,
    B_x: jax.Array,
    B_w1: jax.Array,
    B_w2: jax.Array,
    B_w3: jax.Array,
    B_w4: jax.Array,
):
    del B_x
    x = A_x.reshape(S, D)
    beta = A_beta.reshape(1, H)
    any_spec = pl.BlockSpec(memory_space=pl.ANY)
    scratch = [
        pltpu.VMEM((S, D), bf16),
        pltpu.VMEM((D, D), bf16),
        pltpu.VMEM((D, D), bf16),
        pltpu.VMEM((D, D), bf16),
        pltpu.VMEM((2 * D, D), bf16),
        pltpu.VMEM((D, D), bf16),
        pltpu.VMEM((D, D), bf16),
        pltpu.VMEM((D, D), bf16),
        pltpu.VMEM((D, F), bf16),
        pltpu.VMEM((F, D), bf16),
        pltpu.VMEM((1, H), bf16),
        pltpu.VMEM((S, D), f32),
        pltpu.VMEM((S, D), f32),
        pltpu.VMEM((S, D), bf16),
        pltpu.VMEM((S + 2 * HALO, D), f32),
        pltpu.VMEM((L, D), bf16),
        pltpu.VMEM((L, D), bf16),
        pltpu.VMEM((D, L), bf16),
        pltpu.VMEM((D, L), bf16),
        pltpu.VMEM((D, L), bf16),
        pltpu.VMEM((L, D), bf16),
        pltpu.VMEM((NG, MZR, 128), f32),
        pltpu.VMEM((MZR, 128), f32),
        pltpu.VMEM((128, 128), f32),
        pltpu.VMEM((H, 128), f32),
        pltpu.SemaphoreType.DMA((13,)),
        pltpu.SemaphoreType.DMA((S // TB,)),
    ]
    out = pl.pallas_call(
        _kernel,
        out_shape=jax.ShapeDtypeStruct((S, D), bf16),
        in_specs=[any_spec] * 10,
        out_specs=any_spec,
        scratch_shapes=scratch,
        compiler_params=pltpu.CompilerParams(vmem_limit_bytes=112 * 1024 * 1024),
    )(x, A_wq, A_wk, A_wv, A_wo, beta, B_w1, B_w2, B_w3, B_w4)
    return out.reshape(1, S, D)
```

```python
import math

import jax
import jax.numpy as jnp
from jax import lax
import jax.experimental.pallas as pl
import jax.experimental.pallas.tpu as pltpu

f32 = jnp.float32
bf16 = jnp.bfloat16

S = 2048
D = 1024
F = 3584
H = 32
DH = 32
L = 512
NSEG = S // L
NG = D // 128
HC = D // 2
GH = HC // 128
TB = 256
FC = 512
HALO = 8
MZR = 144
EPS = 1e-5
NEG = -1e30
QSCALE = (DH ** -0.5) * math.log2(math.e)
GELU_C0 = math.sqrt(2.0 / math.pi)
GELU_C1 = GELU_C0 * 0.044715
ATT_LAG = 2


def _dot(a, b):
    return jnp.dot(a, b, preferred_element_type=f32)


def _dot_nt(a, b):
    return lax.dot_general(a, b, (((1,), (1,)), ((), ())), preferred_element_type=f32)


def _ln(x):
    m = jnp.mean(x, axis=-1, keepdims=True)
    xc = x - m
    v = jnp.mean(xc * xc, axis=-1, keepdims=True)
    return xc * lax.rsqrt(v + EPS)


def _gelu(x):
    t = jnp.tanh(x * (GELU_C0 + GELU_C1 * (x * x)))
    hx = 0.5 * x
    return hx + hx * t


def _phi(t):
    return jnp.where(t > 0, t + 1.0, jnp.exp(t))


def _fold(x, op):
    parts = [x[8 * i:8 * i + 8] for i in range(x.shape[0] // 8)]
    while len(parts) > 1:
        parts = [op(parts[i], parts[i + 1]) for i in range(0, len(parts), 2)]
    return parts[0]


def _attention(k_ref, qt_ref, pqt_ref, vt_ref, mz_ref, g0, gate_ref, mask_ref, o_ref, hooks):
    steps = [(g, j, t) for g in range(GH) for j in range(4) for t in range(j + 1)]
    scores, run, mem, outs = {}, {}, {}, {}

    def do_qk(n):
        g, j, t = steps[n]
        if j == 0:
            mem[g] = _dot(mz_ref[g0 + g].astype(bf16), pqt_ref[128 * g:128 * g + 128, :])
        cols = []
        for h in range(4):
            r0 = 128 * g + 32 * h
            parts = []
            if h > 0:
                parts.append(jnp.zeros((32 * h, 128), bf16))
            parts.append(qt_ref[r0:r0 + 32, 128 * j:128 * j + 128])
            if h < 3:
                parts.append(jnp.zeros((96 - 32 * h, 128), bf16))
            cols.append(jnp.concatenate(parts, axis=0))
        w = jnp.concatenate(cols, axis=1)
        scores[n] = _dot(k_ref[128 * t:128 * t + 128, 128 * g:128 * g + 128], w)

    def do_sm(n):
        g, j, t = steps[n]
        st = scores.pop(n)
        cur = []
        for h in range(4):
            s = st[:, 128 * h:128 * h + 128]
            if t == j:
                s = s + mask_ref[...]
            m = jnp.max(_fold(s, jnp.maximum), axis=0, keepdims=True)
            if t > 0:
                m = jnp.maximum(m, run[h][0])
            cur.append((s, m))
        res = []
        for h in range(4):
            s, m = cur[h]
            r0 = 128 * g + 32 * h
            p = jnp.exp2(s - m)
            sm = _fold(p, jnp.add)
            o = _dot(vt_ref[r0:r0 + 32, 128 * t:128 * t + 128], p.astype(bf16))
            res.append((m, o, sm))
        for h in range(4):
            m, o, sm = res[h]
            if t > 0:
                a = jnp.exp2(run[h][0] - m)
                o = run[h][1] * a + o
                sm = run[h][2] * a + sm
            run[h] = (m, o, sm)
            if t == j:
                gate = gate_ref[4 * g + h:4 * g + h + 1, :]
                l = jnp.sum(sm, axis=0, keepdims=True)
                r = mem[g][:, 128 * j:128 * j + 128]
                den = r[128 + h:129 + h] + 1e-6
                outs[h] = r[32 * h:32 * h + 32] * (gate / den) + o * ((1.0 - gate) / l)
        if t == j:
            ot = jnp.concatenate([outs[h] for h in range(4)], axis=0)
            o_ref[128 * j:128 * j + 128, 128 * g:128 * g + 128] = ot.T.astype(bf16)

    n_steps = len(steps)
    for n in range(n_steps + ATT_LAG):
        if n < n_steps:
            do_qk(n)
        if n in hooks:
            hooks[n]()
        if n >= ATT_LAG:
            do_sm(n - ATT_LAG)


def _kernel(x_hbm, wq_hbm, wk_hbm, wv_hbm, wo_hbm, beta_hbm, w1_hbm, w2_hbm, w3_hbm, w4_hbm,
            out_hbm,
            xio, wqv_s, wk_v, wqvt, wo_v, w1_v, w2_v, w3_v, w4_v, beta_v,
            x_ref, y_ref, xn_ref, h_ref,
            k_ref, pk_ref, qt_ref, pqt_ref, vt_ref, o_ref,
            mz_ref, mzmask_ref, mask_ref, gate_ref,
            sem_in, sem_x, sem_out):
    def cp(src, dst, i):
        return pltpu.make_async_copy(src, dst, sem_in.at[i])

    def x_cp(s):
        r0 = s * L if isinstance(s, int) else pl.multiple_of(s * L, L)
        return pltpu.make_async_copy(x_hbm.at[pl.ds(r0, L)], xio.at[pl.ds(r0, L)], sem_x.at[s])

    def out_cp(t):
        r0 = t * TB if isinstance(t, int) else pl.multiple_of(t * TB, TB)
        return pltpu.make_async_copy(xio.at[pl.ds(r0, TB)], out_hbm.at[pl.ds(r0, TB)], sem_out.at[t])

    wqv_cp = [cp(w.at[:, pl.ds(HC * a, HC)], wqv_s.at[2 * a + i], 2 * a + i)
              for a in range(2) for i, w in enumerate((wq_hbm, wv_hbm))]
    wk_cp = [cp(wk_hbm.at[:, pl.ds(HC * a, HC)], wk_v.at[a], 4 + a) for a in range(2)]
    beta_cp = cp(beta_hbm, beta_v, 6)
    wo_cp = cp(wo_hbm, wo_v, 7)
    w1_cp = cp(w1_hbm, w1_v, 8)
    w2_cp = cp(w2_hbm, w2_v, 9)
    w3_cp = cp(w3_hbm, w3_v, 10)
    w4_cp = cp(w4_hbm, w4_v, 11)

    for c in [beta_cp, x_cp(0)] + wqv_cp + wk_cp:
        c.start()

    kk = lax.broadcasted_iota(jnp.int32, (128, 128), 0)
    qq = lax.broadcasted_iota(jnp.int32, (128, 128), 1)
    mask_ref[...] = jnp.where(kk <= qq, 0.0, NEG).astype(f32)
    rr = lax.broadcasted_iota(jnp.int32, (MZR, 128), 0)
    cc = lax.broadcasted_iota(jnp.int32, (MZR, 128), 1) // DH
    row_head = jnp.where(rr < 128, rr // DH, rr - 128)
    mzmask_ref[...] = jnp.where(row_head == cc, 1.0, 0.0).astype(f32)
    h_ref[0:HALO, :] = jnp.zeros((HALO, D), f32)
    h_ref[HALO + S:HALO + S + HALO, :] = jnp.zeros((HALO, D), f32)

    beta_cp.wait()
    eye = (lax.broadcasted_iota(jnp.int32, (H, H), 0) == lax.broadcasted_iota(jnp.int32, (H, H), 1))
    beta_rows = jnp.broadcast_to(beta_v[...].astype(f32), (H, H))
    beta_col = jnp.sum(jnp.where(eye, beta_rows, 0.0), axis=1, keepdims=True)
    gates = jnp.broadcast_to(jax.nn.sigmoid(beta_col), (H, 128))
    gate_ref[0] = gates[0:H // 2]
    gate_ref[1] = gates[H // 2:H]

    def norm_rows(layer, r0):
        rows = pl.ds(pl.multiple_of(r0, TB), TB)
        xv = jnp.where(layer == 0, xio[rows, :].astype(f32), x_ref[rows, :])
        x_ref[rows, :] = xv
        xn_ref[rows, :] = _ln(xv).astype(bf16)

    def pt_body(layer, u):
        s = u // 2
        a = u % 2

        @pl.when(jnp.logical_and(layer == 0, jnp.logical_and(a == 0, s < NSEG - 1)))
        def _():
            x_cp(s + 1).wait()

        r0 = pl.multiple_of(s * L, L)
        xn = xn_ref[pl.ds(r0, L), :]
        norm_rows(layer, jnp.minimum(s + 1, NSEG - 1) * L + a * TB)
        qf = _dot_nt(wqvt[2 * a], xn)
        qt_ref[...] = (qf * QSCALE).astype(bf16)
        pqt_ref[...] = _phi(qf).astype(bf16)
        kf = _dot(xn, wk_v[a])
        k_ref[...] = kf.astype(bf16)
        pk_ref[...] = _phi(kf).astype(bf16)

        def v_proj(c):
            rs = slice(256 * c, 256 * c + 256)
            vt_ref[rs, :] = _dot_nt(wqvt[2 * a + 1, rs, :], xn).astype(bf16)

        v_proj(0)
        g0 = GH * a
        _attention(k_ref, qt_ref, pqt_ref, vt_ref, mz_ref, g0, gate_ref.at[a], mask_ref,
                   o_ref.at[a, pl.ds(r0, L)], {ATT_LAG - 1: lambda: v_proj(1)})

        ones = jnp.ones((MZR - 128, L), bf16)
        for g in range(GH):
            lhs = jnp.concatenate([vt_ref[128 * g:128 * g + 128, :], ones], axis=0)
            upd = _dot(lhs, pk_ref[:, 128 * g:128 * g + 128])
            mz_ref[g0 + g] = mz_ref[g0 + g] + upd * mzmask_ref[...]

    def out_body(t):
        r0 = pl.multiple_of(t * TB, TB)
        half = TB // 2
        yn = []
        for a in range(2):
            rows = pl.ds(pl.multiple_of(r0 + half * a, half), half)
            ov = jnp.concatenate([o_ref[0, rows, :], o_ref[1, rows, :]], axis=1)
            xv = x_ref[rows, :] + _dot(ov, wo_v[...])
            x_ref[rows, :] = xv
            y = _ln(xv)
            y_ref[rows, :] = y
            yn.append(_ln(y).astype(bf16))
        for a in range(2):
            rows = pl.ds(pl.multiple_of(r0 + half * a + HALO, 8), half)
            h_ref[rows, :] = _gelu(_dot(yn[a], w1_v[...]))

    def mix_body(layer, t):
        r0 = pl.multiple_of(t * TB, TB)
        half = TB // 2
        c4 = D // 4
        x1n, xr = [], []
        for a in range(2):
            ra = pl.multiple_of(r0 + half * a, half)
            win = h_ref[pl.ds(ra, half + 2 * HALO), :]
            hs_in = jnp.concatenate([
                win[HALO - 1:HALO - 1 + half, 0 * c4:1 * c4],
                win[HALO + 1:HALO + 1 + half, 1 * c4:2 * c4],
                win[HALO - 2:HALO - 2 + half, 2 * c4:3 * c4],
                win[HALO + 2:HALO + 2 + half, 3 * c4:4 * c4]], axis=1).astype(bf16)
            x1 = y_ref[pl.ds(ra, half), :] + _dot(hs_in, w2_v[...])
            xr.append(x_ref[pl.ds(ra, half), :] + x1)
            x1n.append(_ln(x1).astype(bf16))
        nch = F // FC
        x1n_full = jnp.concatenate(x1n, axis=0)

        def up(c):
            w = w3_v[:, FC * c:FC * c + FC]
            if c == 0:
                return jnp.concatenate([_gelu(_dot(x1n[a], w)) for a in range(2)], axis=0).astype(bf16)
            return _gelu(_dot(x1n_full, w)).astype(bf16)

        acc = jnp.concatenate(xr, axis=0)
        hcur = up(0)
        for c in range(nch):
            hnext = up(c + 1) if c + 1 < nch else None
            acc = acc + _dot(hcur, w4_v[FC * c:FC * c + FC, :])
            hcur = hnext
        x_ref[pl.ds(r0, TB), :] = acc
        xio[pl.ds(r0, TB), :] = acc.astype(bf16)

        @pl.when(layer == 1)
        def _():
            out_cp(t).start()

    def loop(n, fn, name):
        def body(i, c):
            with jax.named_scope(name):
                fn(i)
            return c

        lax.fori_loop(0, n, body, 0)

    def layer_body(layer):
        mz_ref[...] = jnp.zeros(mz_ref.shape, f32)

        @pl.when(layer == 0)
        def _():
            x_cp(0).wait()

        loop(L // TB, lambda i: norm_rows(layer, i * TB), "norm0")

        @pl.when(layer == 0)
        def _():
            def tr(i):
                pltpu.make_async_copy(wqv_s.at[i], wqv_s.at[i], sem_in.at[i]).wait()
                wqvt[i] = wqv_s[i].T

            loop(4, tr, "transpose")
            for c in wk_cp:
                c.wait()
            for c in [x_cp(s) for s in range(1, NSEG)] + [wo_cp, w1_cp, w2_cp, w3_cp, w4_cp]:
                c.start()

        loop(2 * NSEG, lambda u: pt_body(layer, u), "pt")

        @pl.when(layer == 0)
        def _():
            wo_cp.wait()
            w1_cp.wait()

        loop(S // TB, out_body, "out")

        @pl.when(layer == 0)
        def _():
            w2_cp.wait()
            w3_cp.wait()
            w4_cp.wait()

        loop(S // TB, lambda t: mix_body(layer, t), "mix")

    loop(2, layer_body, "layer")
    for t in range(S // TB):
        out_cp(t).wait()


@jax.jit
def pallas_interleave_layers__memory_aug_infini_attn__mixer_s_mlp__prompt_kernel(
    A_x: jax.Array,
    A_wq: jax.Array,
    A_wk: jax.Array,
    A_wv: jax.Array,
    A_wo: jax.Array,
    A_beta: jax.Array,
    B_x: jax.Array,
    B_w1: jax.Array,
    B_w2: jax.Array,
    B_w3: jax.Array,
    B_w4: jax.Array,
):
    del B_x
    x = A_x.reshape(S, D)
    beta = A_beta.reshape(1, H)
    any_spec = pl.BlockSpec(memory_space=pl.ANY)
    scratch = [
        pltpu.VMEM((S, D), bf16),
        pltpu.VMEM((4, D, HC), bf16),
        pltpu.VMEM((2, D, HC), bf16),
        pltpu.VMEM((4, HC, D), bf16),
        pltpu.VMEM((D, D), bf16),
        pltpu.VMEM((D, D), bf16),
        pltpu.VMEM((D, D), bf16),
        pltpu.VMEM((D, F), bf16),
        pltpu.VMEM((F, D), bf16),
        pltpu.VMEM((1, H), bf16),
        pltpu.VMEM((S, D), f32),
        pltpu.VMEM((S, D), f32),
        pltpu.VMEM((S, D), bf16),
        pltpu.VMEM((S + 2 * HALO, D), f32),
        pltpu.VMEM((L, HC), bf16),
        pltpu.VMEM((L, HC), bf16),
        pltpu.VMEM((HC, L), bf16),
        pltpu.VMEM((HC, L), bf16),
        pltpu.VMEM((HC, L), bf16),
        pltpu.VMEM((2, S, HC), bf16),
        pltpu.VMEM((NG, MZR, 128), f32),
        pltpu.VMEM((MZR, 128), f32),
        pltpu.VMEM((128, 128), f32),
        pltpu.VMEM((2, H // 2, 128), f32),
        pltpu.SemaphoreType.DMA((12,)),
        pltpu.SemaphoreType.DMA((NSEG,)),
        pltpu.SemaphoreType.DMA((S // TB,)),
    ]
    out = pl.pallas_call(
        _kernel,
        out_shape=jax.ShapeDtypeStruct((S, D), bf16),
        in_specs=[any_spec] * 10,
        out_specs=any_spec,
        scratch_shapes=scratch,
        compiler_params=pltpu.CompilerParams(vmem_limit_bytes=112 * 1024 * 1024),
    )(x, A_wq, A_wk, A_wv, A_wo, beta, B_w1, B_w2, B_w3, B_w4)
    return out.reshape(1, S, D)
```

```python
import functools
import math

import jax
import jax.numpy as jnp
from jax import lax
import jax.experimental.pallas as pl
import jax.experimental.pallas.tpu as pltpu

f32 = jnp.float32
bf16 = jnp.bfloat16

S = 2048
D = 1024
F = 3584
H = 32
DH = 32
L = 512
NSEG = S // L
NG = D // 128
HC = D // 2
GH = HC // 128
TB = 256
FC = 512
HALO = 8
MZR = 144
EPS = 1e-5
NEG = -1e30
QSCALE = (DH ** -0.5) * math.log2(math.e)
GELU_C0 = math.sqrt(2.0 / math.pi)
GELU_C1 = GELU_C0 * 0.044715
ATT_LAG = 2
QV_STEPS = (-9, -7, -5, -4)
K_STEPS = (-2, 1)
TAIL = ((33, "mem", 0), (35, "mem", 1), (37, "mem", 2), (39, "k", 0), (42, "k", 1), (42, "mem", 3))


def _dot(a, b):
    return jnp.dot(a, b, preferred_element_type=f32)


def _dot_nt(a, b):
    return lax.dot_general(a, b, (((1,), (1,)), ((), ())), preferred_element_type=f32)


def _ln(x):
    m = jnp.mean(x, axis=-1, keepdims=True)
    xc = x - m
    v = jnp.mean(xc * xc, axis=-1, keepdims=True)
    return xc * lax.rsqrt(v + EPS)


def _gelu(x):
    t = jnp.tanh(x * (GELU_C0 + GELU_C1 * (x * x)))
    hx = 0.5 * x
    return hx + hx * t


def _phi(t):
    return jnp.where(t > 0, t + 1.0, jnp.exp(t))


def _fold(x, op):
    parts = [x[8 * i:8 * i + 8] for i in range(x.shape[0] // 8)]
    while len(parts) > 1:
        parts = [op(parts[i], parts[i + 1]) for i in range(0, len(parts), 2)]
    return parts[0]


def _attention(k_ref, qt_ref, pqt_ref, vt_ref, mz_ref, g0, gate_ref, mask_ref, zero_ref, o_ref, hooks):
    steps = [(g, j, t) for g in range(GH) for j in range(4) for t in range(j + 1)]
    scores, run, mem, outs = {}, {}, {}, {}
    drained = []

    def do_qk(n):
        g, j, t = steps[n]
        if j == 0:
            mem[g] = _dot(mz_ref[g0 + g].astype(bf16), pqt_ref[128 * g:128 * g + 128, :])
        cols = []
        for h in range(4):
            r0 = 128 * g + 32 * h
            parts = []
            if h > 0:
                parts.append(jnp.zeros((32 * h, 128), bf16))
            parts.append(qt_ref[r0:r0 + 32, 128 * j:128 * j + 128])
            if h < 3:
                parts.append(jnp.zeros((96 - 32 * h, 128), bf16))
            cols.append(jnp.concatenate(parts, axis=0))
        w = jnp.concatenate(cols, axis=1)
        scores[n] = _dot(k_ref[128 * t:128 * t + 128, 128 * g:128 * g + 128], w)

    def do_sm(n):
        g, j, t = steps[n]
        st = scores.pop(n)
        cur = []
        for h in range(4):
            s = st[:, 128 * h:128 * h + 128]
            if t == j:
                s = s + mask_ref[...]
            m = jnp.max(_fold(s, jnp.maximum), axis=0, keepdims=True)
            if t > 0:
                m = jnp.maximum(m, run[h][0])
            cur.append((s, m))
        res = []
        for h in range(4):
            s, m = cur[h]
            r0 = 128 * g + 32 * h
            p = jnp.exp2(s - m)
            sm = _fold(p, jnp.add)
            o = _dot(vt_ref[r0:r0 + 32, 128 * t:128 * t + 128], p.astype(bf16))
            res.append((m, o, sm))
        for h in range(4):
            m, o, sm = res[h]
            if t > 0:
                a = jnp.exp2(run[h][0] - m)
                o = run[h][1] * a + o
                sm = run[h][2] * a + sm
            run[h] = (m, o, sm)
            if t == j:
                gate = gate_ref[4 * g + h:4 * g + h + 1, :]
                if drained:
                    sm = pltpu.bitcast(pltpu.bitcast(sm, jnp.uint32) | drained.pop(), f32)
                l = jnp.sum(sm, axis=0, keepdims=True)
                r = mem[g][:, 128 * j:128 * j + 128]
                den = r[128 + h:129 + h] + 1e-6
                outs[h] = r[32 * h:32 * h + 32] * (gate / den) + o * ((1.0 - gate) / l)
        if t == j:
            ot = jnp.concatenate([outs[h] for h in range(4)], axis=0)
            ob = ot.T.astype(bf16)
            o_ref[128 * j:128 * j + 128, 128 * g:128 * g + 128] = ob
            drained.append(pltpu.bitcast(ob[112:128], jnp.uint32) & zero_ref[...])

    n_steps = len(steps)
    for n in range(n_steps + ATT_LAG):
        if n < n_steps:
            do_qk(n)
        for p in hooks.get(n, []):
            p()
        if n >= ATT_LAG:
            do_sm(n - ATT_LAG)
    for p in hooks.get(n_steps + ATT_LAG, []):
        p()


def _kernel(x_hbm, wq_hbm, wk_hbm, wv_hbm, wo_hbm, beta_hbm, w1_hbm, w2_hbm, w3_hbm, w4_hbm,
            out_hbm,
            xio, wqv_s, wk_v, wqvt, wo_v, w1_v, w2_v, w3_v, w4_v, beta_v,
            x_ref, y_ref, xn_ref, xc_ref, h_ref,
            k_ref, pk_ref, qt_ref, pqt_ref, vt_ref, o_ref,
            mz_ref, mzmask_ref, mask_ref, gate_ref, zero_ref,
            sem_in, sem_x, sem_out):
    def cp(src, dst, i):
        return pltpu.make_async_copy(src, dst, sem_in.at[i])

    def x_cp(t):
        r0 = t * TB if isinstance(t, int) else pl.multiple_of(t * TB, TB)
        return pltpu.make_async_copy(x_hbm.at[pl.ds(r0, TB)], xio.at[pl.ds(r0, TB)], sem_x.at[t])

    def out_cp(t):
        r0 = t * TB if isinstance(t, int) else pl.multiple_of(t * TB, TB)
        return pltpu.make_async_copy(xio.at[pl.ds(r0, TB)], out_hbm.at[pl.ds(r0, TB)], sem_out.at[t])

    wqv_cp = [cp(w.at[:, pl.ds(HC * a, HC)], wqv_s.at[2 * a + i], 2 * a + i)
              for a in range(2) for i, w in enumerate((wq_hbm, wv_hbm))]
    wk0_cp = cp(wk_hbm.at[:, pl.ds(0, HC)], wk_v.at[0], 4)
    wk1a_cp = cp(wk_hbm.at[:, pl.ds(HC, 128)], wk_v.at[1, :, pl.ds(0, 128)], 5)
    wk1b_cp = cp(wk_hbm.at[:, pl.ds(HC + 128, HC - 128)], wk_v.at[1, :, pl.ds(128, HC - 128)], 12)
    beta_cp = cp(beta_hbm, beta_v, 6)
    wo_cp = cp(wo_hbm, wo_v, 7)
    w1_cp = cp(w1_hbm, w1_v, 8)
    w2_cp = cp(w2_hbm, w2_v, 9)
    w3_cp = cp(w3_hbm, w3_v, 10)
    w4_cp = cp(w4_hbm, w4_v, 11)

    for c in [beta_cp, x_cp(0), x_cp(1), wk0_cp]:
        c.start()

    kk = lax.broadcasted_iota(jnp.int32, (128, 128), 0)
    qq = lax.broadcasted_iota(jnp.int32, (128, 128), 1)
    mask_ref[...] = jnp.where(kk <= qq, 0.0, NEG).astype(f32)
    rr = lax.broadcasted_iota(jnp.int32, (MZR, 128), 0)
    cc = lax.broadcasted_iota(jnp.int32, (MZR, 128), 1) // DH
    row_head = jnp.where(rr < 128, rr // DH, rr - 128)
    mzmask_ref[...] = jnp.where(row_head == cc, 1.0, 0.0).astype(f32)
    zero_ref[...] = jnp.zeros((8, 128), jnp.uint32)
    h_ref[0:HALO, :] = jnp.zeros((HALO, D), f32)
    h_ref[HALO + S:HALO + S + HALO, :] = jnp.zeros((HALO, D), f32)

    beta_cp.wait()
    eye = (lax.broadcasted_iota(jnp.int32, (H, H), 0) == lax.broadcasted_iota(jnp.int32, (H, H), 1))
    beta_rows = jnp.broadcast_to(beta_v[...].astype(f32), (H, H))
    beta_col = jnp.sum(jnp.where(eye, beta_rows, 0.0), axis=1, keepdims=True)
    gates = jnp.broadcast_to(jax.nn.sigmoid(beta_col), (H, 128))
    gate_ref[0] = gates[0:H // 2]
    gate_ref[1] = gates[H // 2:H]

    def loop(n, fn, name):
        def body(i, c):
            with jax.named_scope(name):
                fn(i)
            return c

        lax.fori_loop(0, n, body, 0)

    def norm_rows(layer, r0):
        rows = pl.ds(pl.multiple_of(r0, TB), TB)
        xv = jnp.where(layer == 0, xio[rows, :].astype(f32), x_ref[rows, :])
        x_ref[rows, :] = xv
        xn_ref[rows, :] = _ln(xv).astype(bf16)

    def k_store(kf, g, c):
        gs, rs = slice(128 * g, 128 * g + 128), slice(256 * c, 256 * c + 256)
        k_ref[rs, gs] = kf.astype(bf16)
        pk_ref[rs, gs] = _phi(kf).astype(bf16)

    def k_first(u, c):
        r0 = (u // 2) * L + 256 * c
        rows = pl.ds(r0 if isinstance(u, int) else pl.multiple_of(r0, 256), 256)
        k_store(_dot(xn_ref[rows, :], wk_v[u % 2, :, 0:128]), 0, c)

    def pt_body(layer, u):
        s = u // 2
        a = u % 2

        @pl.when(jnp.logical_and(layer == 0, u < 2))
        def _():
            def tr(i):
                src = wqv_s.at[2 * u + i]
                pltpu.make_async_copy(src, src, sem_in.at[2 * u + i]).wait()
                wt = src[...].T
                for g in range(GH):
                    wqvt[u, g, pl.ds(pl.multiple_of(128 * i, 128), 128), :] = wt[128 * g:128 * g + 128]

            loop(2, tr, "transpose")

            @pl.when(u == 0)
            def _():
                wk1a_cp.wait()
                for c in [wqv_cp[2], wqv_cp[3], wk1b_cp, x_cp(3)]:
                    c.start()

            @pl.when(u == 1)
            def _():
                wk1b_cp.wait()
                for c in [x_cp(t) for t in range(4, S // TB)] + [wo_cp, w1_cp, w2_cp, w3_cp, w4_cp]:
                    c.start()

        @pl.when(jnp.logical_and(layer == 0, u < S // TB - 2))
        def _():
            x_cp(u + 2).wait()

        r0 = pl.multiple_of(s * L, L)
        xc_ref[...] = xn_ref[pl.ds(r0, L), :]
        norm_rows(layer, jnp.minimum(s + 1, NSEG - 1) * L + a * TB)
        g0 = GH * a

        def qv_proj(g, c):
            gs, cs = slice(128 * g, 128 * g + 128), slice(128 * c, 128 * c + 128)
            r = _dot_nt(wqvt[a, g], xc_ref[cs, :])
            qt_ref[gs, cs] = (r[0:128] * QSCALE).astype(bf16)
            pqt_ref[gs, cs] = _phi(r[0:128]).astype(bf16)
            vt_ref[gs, cs] = r[128:256].astype(bf16)

        def k_proj(g, c):
            k_store(_dot(xc_ref[256 * c:256 * c + 256, :], wk_v[a, :, 128 * g:128 * g + 128]), g, c)

        def mem_update(g):
            ones = jnp.ones((MZR - 128, L), bf16)
            lhs = jnp.concatenate([vt_ref[128 * g:128 * g + 128, :], ones], axis=0)
            upd = _dot(lhs, pk_ref[:, 128 * g:128 * g + 128])
            mz_ref[g0 + g] = mz_ref[g0 + g] + upd * mzmask_ref[...]

        hooks = {}

        def at(n, fn, *args):
            hooks.setdefault(max(n, -1), []).append(functools.partial(fn, *args))

        for g in range(GH):
            for c in range(4):
                at(10 * g + QV_STEPS[c], qv_proj, g, c)
            for c in range(2):
                if g > 0:
                    at(10 * g + K_STEPS[c], k_proj, g, c)
        u_next = jnp.minimum(u + 1, 2 * NSEG - 1)
        for n, kind, i in TAIL:
            if kind == "mem":
                at(n, mem_update, i)
            else:
                at(n, k_first, u_next, i)
        for p in hooks.pop(-1):
            p()
        _attention(k_ref, qt_ref, pqt_ref, vt_ref, mz_ref, g0, gate_ref.at[a], mask_ref, zero_ref,
                   o_ref.at[a, pl.ds(r0, L)], hooks)

    def out_body(t):
        r0 = pl.multiple_of(t * TB, TB)
        half = TB // 2
        yn = []
        for a in range(2):
            rows = pl.ds(pl.multiple_of(r0 + half * a, half), half)
            ov = jnp.concatenate([o_ref[0, rows, :], o_ref[1, rows, :]], axis=1)
            xv = x_ref[rows, :] + _dot(ov, wo_v[...])
            x_ref[rows, :] = xv
            y = _ln(xv)
            y_ref[rows, :] = y
            yn.append(_ln(y).astype(bf16))
        for a in range(2):
            rows = pl.ds(pl.multiple_of(r0 + half * a + HALO, 8), half)
            h_ref[rows, :] = _gelu(_dot(yn[a], w1_v[...]))

    def mix_body(layer, t):
        r0 = pl.multiple_of(t * TB, TB)
        half = TB // 2
        c4 = D // 4
        x1n, xr = [], []
        for a in range(2):
            ra = pl.multiple_of(r0 + half * a, half)
            win = h_ref[pl.ds(ra, half + 2 * HALO), :]
            hs_in = jnp.concatenate([
                win[HALO - 1:HALO - 1 + half, 0 * c4:1 * c4],
                win[HALO + 1:HALO + 1 + half, 1 * c4:2 * c4],
                win[HALO - 2:HALO - 2 + half, 2 * c4:3 * c4],
                win[HALO + 2:HALO + 2 + half, 3 * c4:4 * c4]], axis=1).astype(bf16)
            x1 = y_ref[pl.ds(ra, half), :] + _dot(hs_in, w2_v[...])
            xr.append(x_ref[pl.ds(ra, half), :] + x1)
            x1n.append(_ln(x1).astype(bf16))
        nch = F // FC
        x1n_full = jnp.concatenate(x1n, axis=0)

        def up(c):
            w = w3_v[:, FC * c:FC * c + FC]
            if c == 0:
                return jnp.concatenate([_gelu(_dot(x1n[a], w)) for a in range(2)], axis=0).astype(bf16)
            return _gelu(_dot(x1n_full, w)).astype(bf16)

        acc = jnp.concatenate(xr, axis=0)
        hcur = up(0)
        for c in range(nch):
            hnext = up(c + 1) if c + 1 < nch else None
            acc = acc + _dot(hcur, w4_v[FC * c:FC * c + FC, :])
            hcur = hnext
        x_ref[pl.ds(r0, TB), :] = acc
        xio[pl.ds(r0, TB), :] = acc.astype(bf16)

        @pl.when(layer == 1)
        def _():
            out_cp(t).start()

    def layer_body(layer):
        mz_ref[...] = jnp.zeros(mz_ref.shape, f32)

        def norm0(i):
            @pl.when(layer == 0)
            def _():
                x_cp(i).wait()

                @pl.when(i == 0)
                def _():
                    wqv_cp[0].start()

                @pl.when(i == 1)
                def _():
                    wqv_cp[1].start()

            norm_rows(layer, i * TB)

        loop(L // TB, norm0, "norm0")

        @pl.when(layer == 0)
        def _():
            wk0_cp.wait()
            x_cp(2).start()
            wk1a_cp.start()

        for c in range(2):
            k_first(0, c)
        loop(2 * NSEG, lambda u: pt_body(layer, u), "pt")

        @pl.when(layer == 0)
        def _():
            wo_cp.wait()
            w1_cp.wait()

        loop(S // TB, out_body, "out")

        @pl.when(layer == 0)
        def _():
            w2_cp.wait()
            w3_cp.wait()
            w4_cp.wait()

        loop(S // TB, lambda t: mix_body(layer, t), "mix")

    loop(2, layer_body, "layer")
    for t in range(S // TB):
        out_cp(t).wait()


@jax.jit
def pallas_interleave_layers__memory_aug_infini_attn__mixer_s_mlp__prompt_kernel(
    A_x: jax.Array,
    A_wq: jax.Array,
    A_wk: jax.Array,
    A_wv: jax.Array,
    A_wo: jax.Array,
    A_beta: jax.Array,
    B_x: jax.Array,
    B_w1: jax.Array,
    B_w2: jax.Array,
    B_w3: jax.Array,
    B_w4: jax.Array,
):
    del B_x
    x = A_x.reshape(S, D)
    beta = A_beta.reshape(1, H)
    any_spec = pl.BlockSpec(memory_space=pl.ANY)
    scratch = [
        pltpu.VMEM((S, D), bf16),
        pltpu.VMEM((4, D, HC), bf16),
        pltpu.VMEM((2, D, HC), bf16),
        pltpu.VMEM((2, GH, 256, D), bf16),
        pltpu.VMEM((D, D), bf16),
        pltpu.VMEM((D, D), bf16),
        pltpu.VMEM((D, D), bf16),
        pltpu.VMEM((D, F), bf16),
        pltpu.VMEM((F, D), bf16),
        pltpu.VMEM((1, H), bf16),
        pltpu.VMEM((S, D), f32),
        pltpu.VMEM((S, D), f32),
        pltpu.VMEM((S, D), bf16),
        pltpu.VMEM((L, D), bf16),
        pltpu.VMEM((S + 2 * HALO, D), f32),
        pltpu.VMEM((L, HC), bf16),
        pltpu.VMEM((L, HC), bf16),
        pltpu.VMEM((HC, L), bf16),
        pltpu.VMEM((HC, L), bf16),
        pltpu.VMEM((HC, L), bf16),
        pltpu.VMEM((2, S, HC), bf16),
        pltpu.VMEM((NG, MZR, 128), f32),
        pltpu.VMEM((MZR, 128), f32),
        pltpu.VMEM((128, 128), f32),
        pltpu.VMEM((2, H // 2, 128), f32),
        pltpu.VMEM((8, 128), jnp.uint32),
        pltpu.SemaphoreType.DMA((13,)),
        pltpu.SemaphoreType.DMA((S // TB,)),
        pltpu.SemaphoreType.DMA((S // TB,)),
    ]
    out = pl.pallas_call(
        _kernel,
        out_shape=jax.ShapeDtypeStruct((S, D), bf16),
        in_specs=[any_spec] * 10,
        out_specs=any_spec,
        scratch_shapes=scratch,
        compiler_params=pltpu.CompilerParams(vmem_limit_bytes=112 * 1024 * 1024),
    )(x, A_wq, A_wk, A_wv, A_wo, beta, B_w1, B_w2, B_w3, B_w4)
    return out.reshape(1, S, D)
```

```python
import functools
import math

import jax
import jax.numpy as jnp
from jax import lax
import jax.experimental.pallas as pl
import jax.experimental.pallas.tpu as pltpu

f32 = jnp.float32
bf16 = jnp.bfloat16

S = 2048
D = 1024
F = 3584
H = 32
DH = 32
L = 512
NSEG = S // L
NG = D // 128
HC = D // 2
GH = HC // 128
TB = 256
FC = 512
HALO = 8
MZR = 144
EPS = 1e-5
NEG = -1e30
QSCALE = (DH ** -0.5) * math.log2(math.e)
GELU_C0 = math.sqrt(2.0 / math.pi)
GELU_C1 = GELU_C0 * 0.044715
ATT_LAG = 2
LNC = 16
QV_STEPS = (-9, -7, -5, -4)
K_STEPS = (-2, 1)
TAIL = ((33, "mem", 0), (35, "mem", 1), (37, "mem", 2), (39, "k", 0), (42, "k", 1), (42, "mem", 3))


def _dot(a, b):
    return jnp.dot(a, b, preferred_element_type=f32)


def _dot_nt(a, b):
    return lax.dot_general(a, b, (((1,), (1,)), ((), ())), preferred_element_type=f32)


def _ln(x):
    m = jnp.mean(x, axis=-1, keepdims=True)
    xc = x - m
    v = jnp.mean(xc * xc, axis=-1, keepdims=True)
    return xc * lax.rsqrt(v + EPS)


def _ln_chunks(mean, load, zero, post):
    outs, prev = [], None
    for i in range(mean.shape[0] // LNC):
        m = mean[LNC * i:LNC * i + LNC]
        if prev is not None:
            m = pltpu.bitcast(pltpu.bitcast(m, jnp.int32) | (pltpu.bitcast(prev, jnp.int32) & zero), f32)
        xc = load(i) - m
        prev = lax.rsqrt(jnp.mean(xc * xc, axis=-1, keepdims=True) + EPS)
        outs.append(post(i, xc * prev))
    return outs


def _rowmean(x):
    return jnp.mean(x, axis=-1, keepdims=True)


def _gelu(x):
    t = jnp.tanh(x * (GELU_C0 + GELU_C1 * (x * x)))
    hx = 0.5 * x
    return hx + hx * t


def _phi(t):
    return jnp.where(t > 0, t + 1.0, jnp.exp(t))


def _fold(x, op):
    parts = [x[8 * i:8 * i + 8] for i in range(x.shape[0] // 8)]
    while len(parts) > 1:
        parts = [op(parts[i], parts[i + 1]) for i in range(0, len(parts), 2)]
    return parts[0]


def _attention(k_ref, qt_ref, pqt_ref, vt_ref, mz_ref, g0, gate_ref, mask_ref, zero_ref, o_ref, hooks):
    steps = [(g, j, t) for g in range(GH) for j in range(4) for t in range(j + 1)]
    scores, run, mem, outs = {}, {}, {}, {}
    drained = []

    def do_qk(n):
        g, j, t = steps[n]
        if j == 0:
            mem[g] = _dot(mz_ref[g0 + g].astype(bf16), pqt_ref[128 * g:128 * g + 128, :])
        cols = []
        for h in range(4):
            r0 = 128 * g + 32 * h
            parts = []
            if h > 0:
                parts.append(jnp.zeros((32 * h, 128), bf16))
            parts.append(qt_ref[r0:r0 + 32, 128 * j:128 * j + 128])
            if h < 3:
                parts.append(jnp.zeros((96 - 32 * h, 128), bf16))
            cols.append(jnp.concatenate(parts, axis=0))
        w = jnp.concatenate(cols, axis=1)
        scores[n] = _dot(k_ref[128 * t:128 * t + 128, 128 * g:128 * g + 128], w)

    def do_sm(n):
        g, j, t = steps[n]
        st = scores.pop(n)
        cur = []
        for h in range(4):
            s = st[:, 128 * h:128 * h + 128]
            if t == j:
                s = s + mask_ref[...]
            m = jnp.max(_fold(s, jnp.maximum), axis=0, keepdims=True)
            if t > 0:
                m = jnp.maximum(m, run[h][0])
            cur.append((s, m))
        res = []
        for h in range(4):
            s, m = cur[h]
            r0 = 128 * g + 32 * h
            p = jnp.exp2(s - m)
            sm = _fold(p, jnp.add)
            o = _dot(vt_ref[r0:r0 + 32, 128 * t:128 * t + 128], p.astype(bf16))
            res.append((m, o, sm))
        for h in range(4):
            m, o, sm = res[h]
            if t > 0:
                a = jnp.exp2(run[h][0] - m)
                o = run[h][1] * a + o
                sm = run[h][2] * a + sm
            run[h] = (m, o, sm)
            if t == j:
                gate = gate_ref[4 * g + h:4 * g + h + 1, :]
                if drained:
                    sm = pltpu.bitcast(pltpu.bitcast(sm, jnp.uint32) | drained.pop(), f32)
                l = jnp.sum(sm, axis=0, keepdims=True)
                r = mem[g][:, 128 * j:128 * j + 128]
                den = r[128 + h:129 + h] + 1e-6
                outs[h] = r[32 * h:32 * h + 32] * (gate / den) + o * ((1.0 - gate) / l)
        if t == j:
            ot = jnp.concatenate([outs[h] for h in range(4)], axis=0)
            ob = ot.T.astype(bf16)
            o_ref[128 * j:128 * j + 128, 128 * g:128 * g + 128] = ob
            drained.append(pltpu.bitcast(ob[112:128], jnp.uint32) & zero_ref[...])

    n_steps = len(steps)
    for n in range(n_steps + ATT_LAG):
        if n < n_steps:
            do_qk(n)
        for p in hooks.get(n, []):
            p()
        if n >= ATT_LAG:
            do_sm(n - ATT_LAG)
    for p in hooks.get(n_steps + ATT_LAG, []):
        p()


def _kernel(x_hbm, wq_hbm, wk_hbm, wv_hbm, wo_hbm, beta_hbm, w1_hbm, w2_hbm, w3_hbm, w4_hbm,
            out_hbm,
            xio, wqv_s, wk_v, wqvt, wo_v, w1_v, w2_v, w3_v, w4_v, beta_v,
            x_ref, y_ref, xn_ref, xc_ref, h_ref,
            k_ref, pk_ref, qt_ref, pqt_ref, vt_ref, o_ref,
            mz_ref, mzmask_ref, mask_ref, gate_ref, zero_ref, zs_ref,
            sem_in, sem_x, sem_out):
    def cp(src, dst, i):
        return pltpu.make_async_copy(src, dst, sem_in.at[i])

    def x_cp(t):
        r0 = t * TB if isinstance(t, int) else pl.multiple_of(t * TB, TB)
        return pltpu.make_async_copy(x_hbm.at[pl.ds(r0, TB)], xio.at[pl.ds(r0, TB)], sem_x.at[t])

    def out_cp(t):
        r0 = t * TB if isinstance(t, int) else pl.multiple_of(t * TB, TB)
        return pltpu.make_async_copy(xio.at[pl.ds(r0, TB)], out_hbm.at[pl.ds(r0, TB)], sem_out.at[t])

    wqv_cp = [cp(w.at[:, pl.ds(HC * a, HC)], wqv_s.at[2 * a + i], 2 * a + i)
              for a in range(2) for i, w in enumerate((wq_hbm, wv_hbm))]
    wk0_cp = cp(wk_hbm.at[:, pl.ds(0, HC)], wk_v.at[0], 4)
    wk1a_cp = cp(wk_hbm.at[:, pl.ds(HC, 128)], wk_v.at[1, :, pl.ds(0, 128)], 5)
    wk1b_cp = cp(wk_hbm.at[:, pl.ds(HC + 128, HC - 128)], wk_v.at[1, :, pl.ds(128, HC - 128)], 12)
    beta_cp = cp(beta_hbm, beta_v, 6)
    wo_cp = cp(wo_hbm, wo_v, 7)
    w1_cp = cp(w1_hbm, w1_v, 8)
    w2_cp = cp(w2_hbm, w2_v, 9)
    w3_cp = cp(w3_hbm, w3_v, 10)
    w4_cp = cp(w4_hbm, w4_v, 11)

    for c in [beta_cp, x_cp(0), x_cp(1), wk0_cp]:
        c.start()

    kk = lax.broadcasted_iota(jnp.int32, (128, 128), 0)
    qq = lax.broadcasted_iota(jnp.int32, (128, 128), 1)
    mask_ref[...] = jnp.where(kk <= qq, 0.0, NEG).astype(f32)
    rr = lax.broadcasted_iota(jnp.int32, (MZR, 128), 0)
    cc = lax.broadcasted_iota(jnp.int32, (MZR, 128), 1) // DH
    row_head = jnp.where(rr < 128, rr // DH, rr - 128)
    mzmask_ref[...] = jnp.where(row_head == cc, 1.0, 0.0).astype(f32)
    zero_ref[...] = jnp.zeros((8, 128), jnp.uint32)
    zs_ref[0] = jnp.int32(0)
    h_ref[0:HALO, :] = jnp.zeros((HALO, D), f32)
    h_ref[HALO + S:HALO + S + HALO, :] = jnp.zeros((HALO, D), f32)

    beta_cp.wait()
    eye = (lax.broadcasted_iota(jnp.int32, (H, H), 0) == lax.broadcasted_iota(jnp.int32, (H, H), 1))
    beta_rows = jnp.broadcast_to(beta_v[...].astype(f32), (H, H))
    beta_col = jnp.sum(jnp.where(eye, beta_rows, 0.0), axis=1, keepdims=True)
    gates = jnp.broadcast_to(jax.nn.sigmoid(beta_col), (H, 128))
    gate_ref[0] = gates[0:H // 2]
    gate_ref[1] = gates[H // 2:H]

    def loop(n, fn, name):
        def body(i, c):
            with jax.named_scope(name):
                fn(i)
            return c

        lax.fori_loop(0, n, body, 0)

    def layer_in(layer, rows):
        return jnp.where(layer == 0, xio[rows, :].astype(f32), x_ref[rows, :])

    def chunk(r0, i):
        return pl.ds(pl.multiple_of(r0 + LNC * i, LNC), LNC)

    def norm_rows(layer, r0, chained=True):
        rows = pl.ds(pl.multiple_of(r0, TB), TB)
        if not chained:
            xn_ref[rows, :] = _ln(layer_in(layer, rows)).astype(bf16)
            return

        def post(i, y):
            xn_ref[chunk(r0, i), :] = y.astype(bf16)

        _ln_chunks(_rowmean(layer_in(layer, rows)), lambda i: layer_in(layer, chunk(r0, i)), zs_ref[0], post)

    def k_store(kf, g, c):
        gs, rs = slice(128 * g, 128 * g + 128), slice(256 * c, 256 * c + 256)
        k_ref[rs, gs] = kf.astype(bf16)
        pk_ref[rs, gs] = _phi(kf).astype(bf16)

    def k_first(u, c):
        r0 = (u // 2) * L + 256 * c
        rows = pl.ds(r0 if isinstance(u, int) else pl.multiple_of(r0, 256), 256)
        k_store(_dot(xn_ref[rows, :], wk_v[u % 2, :, 0:128]), 0, c)

    def pt_body(layer, u):
        s = u // 2
        a = u % 2

        @pl.when(jnp.logical_and(layer == 0, u < 2))
        def _():
            def tr(i):
                src = wqv_s.at[2 * u + i]
                pltpu.make_async_copy(src, src, sem_in.at[2 * u + i]).wait()
                wt = src[...].T
                for g in range(GH):
                    wqvt[u, g, pl.ds(pl.multiple_of(128 * i, 128), 128), :] = wt[128 * g:128 * g + 128]

            loop(2, tr, "transpose")

            @pl.when(u == 0)
            def _():
                wk1a_cp.wait()
                for c in [wqv_cp[2], wqv_cp[3], wk1b_cp, x_cp(3)]:
                    c.start()

            @pl.when(u == 1)
            def _():
                wk1b_cp.wait()
                for c in [x_cp(t) for t in range(4, S // TB)] + [wo_cp, w1_cp, w2_cp, w3_cp, w4_cp]:
                    c.start()

        @pl.when(jnp.logical_and(layer == 0, u < S // TB - 2))
        def _():
            x_cp(u + 2).wait()

        r0 = pl.multiple_of(s * L, L)
        xc_ref[...] = xn_ref[pl.ds(r0, L), :]
        norm_rows(layer, jnp.minimum(s + 1, NSEG - 1) * L + a * TB)
        g0 = GH * a

        def qv_proj(g, c):
            gs, cs = slice(128 * g, 128 * g + 128), slice(128 * c, 128 * c + 128)
            r = _dot_nt(wqvt[a, g], xc_ref[cs, :])
            qt_ref[gs, cs] = (r[0:128] * QSCALE).astype(bf16)
            pqt_ref[gs, cs] = _phi(r[0:128]).astype(bf16)
            vt_ref[gs, cs] = r[128:256].astype(bf16)

        def k_proj(g, c):
            k_store(_dot(xc_ref[256 * c:256 * c + 256, :], wk_v[a, :, 128 * g:128 * g + 128]), g, c)

        def mem_update(g):
            ones = jnp.ones((MZR - 128, L), bf16)
            lhs = jnp.concatenate([vt_ref[128 * g:128 * g + 128, :], ones], axis=0)
            upd = _dot(lhs, pk_ref[:, 128 * g:128 * g + 128])
            mz_ref[g0 + g] = mz_ref[g0 + g] + upd * mzmask_ref[...]

        hooks = {}

        def at(n, fn, *args):
            hooks.setdefault(max(n, -1), []).append(functools.partial(fn, *args))

        for g in range(GH):
            for c in range(4):
                at(10 * g + QV_STEPS[c], qv_proj, g, c)
            for c in range(2):
                if g > 0:
                    at(10 * g + K_STEPS[c], k_proj, g, c)
        u_next = jnp.minimum(u + 1, 2 * NSEG - 1)
        for n, kind, i in TAIL:
            if kind == "mem":
                at(n, mem_update, i)
            else:
                at(n, k_first, u_next, i)
        for p in hooks.pop(-1):
            p()
        _attention(k_ref, qt_ref, pqt_ref, vt_ref, mz_ref, g0, gate_ref.at[a], mask_ref, zero_ref,
                   o_ref.at[a, pl.ds(r0, L)], hooks)

    def out_body(layer, t):
        r0 = pl.multiple_of(t * TB, TB)
        half = TB // 2
        yn = []
        for a in range(2):
            rows = pl.ds(pl.multiple_of(r0 + half * a, half), half)
            ov = jnp.concatenate([o_ref[0, rows, :], o_ref[1, rows, :]], axis=1)
            xv = layer_in(layer, rows) + _dot(ov, wo_v[...])
            x_ref[rows, :] = xv
            y = _ln(xv)
            y_ref[rows, :] = y
            yn.append(_ln(y).astype(bf16))
        for a in range(2):
            rows = pl.ds(pl.multiple_of(r0 + half * a + HALO, 8), half)
            h_ref[rows, :] = _gelu(_dot(yn[a], w1_v[...]))

    def mix_body(layer, t):
        r0 = pl.multiple_of(t * TB, TB)
        half = TB // 2
        c4 = D // 4
        x1n = []
        for a in range(2):
            ra = pl.multiple_of(r0 + half * a, half)
            win = h_ref[pl.ds(ra, half + 2 * HALO), :]
            hs_in = jnp.concatenate([
                win[HALO - 1:HALO - 1 + half, 0 * c4:1 * c4],
                win[HALO + 1:HALO + 1 + half, 1 * c4:2 * c4],
                win[HALO - 2:HALO - 2 + half, 2 * c4:3 * c4],
                win[HALO + 2:HALO + 2 + half, 3 * c4:4 * c4]], axis=1).astype(bf16)
            rows = pl.ds(ra, half)
            x1 = y_ref[rows, :] + _dot(hs_in, w2_v[...])
            y_ref[rows, :] = x1
            xc = y_ref[rows, :] - _rowmean(x1)
            x1n.append((xc * lax.rsqrt(_rowmean(xc * xc) + EPS)).astype(bf16))
        nch = F // FC
        x1n_full = jnp.concatenate(x1n, axis=0)

        def up(lhs, c):
            return _gelu(_dot(lhs, w3_v[:, FC * c:FC * c + FC]))

        hid = {0: jnp.concatenate([up(x1n[a], 0) for a in range(2)], axis=0).astype(bf16)}
        hid[1] = up(x1n_full, 1).astype(bf16)
        acc = x_ref[pl.ds(r0, TB), :] + y_ref[pl.ds(r0, TB), :]
        for c in range(nch):
            acc = acc + _dot(hid.pop(c), w4_v[FC * c:FC * c + FC, :])
            if c + 2 < nch:
                hid[c + 2] = up(x1n_full, c + 2).astype(bf16)
        x_ref[pl.ds(r0, TB), :] = acc
        xio[pl.ds(r0, TB), :] = acc.astype(bf16)

        @pl.when(layer == 1)
        def _():
            out_cp(t).start()

    def layer_body(layer):
        mz_ref[...] = jnp.zeros(mz_ref.shape, f32)

        def norm0(i):
            @pl.when(layer == 0)
            def _():
                x_cp(i).wait()

                @pl.when(i == 0)
                def _():
                    wqv_cp[0].start()

                @pl.when(i == 1)
                def _():
                    wqv_cp[1].start()

            norm_rows(layer, i * TB, chained=False)

        loop(L // TB, norm0, "norm0")

        @pl.when(layer == 0)
        def _():
            wk0_cp.wait()
            x_cp(2).start()
            wk1a_cp.start()

        for c in range(2):
            k_first(0, c)
        loop(2 * NSEG, lambda u: pt_body(layer, u), "pt")

        @pl.when(layer == 0)
        def _():
            wo_cp.wait()
            w1_cp.wait()

        loop(S // TB, lambda t: out_body(layer, t), "out")

        @pl.when(layer == 0)
        def _():
            w2_cp.wait()
            w3_cp.wait()
            w4_cp.wait()

        loop(S // TB, lambda t: mix_body(layer, t), "mix")

    loop(2, layer_body, "layer")
    for t in range(S // TB):
        out_cp(t).wait()


@jax.jit
def pallas_interleave_layers__memory_aug_infini_attn__mixer_s_mlp__prompt_kernel(
    A_x: jax.Array,
    A_wq: jax.Array,
    A_wk: jax.Array,
    A_wv: jax.Array,
    A_wo: jax.Array,
    A_beta: jax.Array,
    B_x: jax.Array,
    B_w1: jax.Array,
    B_w2: jax.Array,
    B_w3: jax.Array,
    B_w4: jax.Array,
):
    del B_x
    x = A_x.reshape(S, D)
    beta = A_beta.reshape(1, H)
    any_spec = pl.BlockSpec(memory_space=pl.ANY)
    scratch = [
        pltpu.VMEM((S, D), bf16),
        pltpu.VMEM((4, D, HC), bf16),
        pltpu.VMEM((2, D, HC), bf16),
        pltpu.VMEM((2, GH, 256, D), bf16),
        pltpu.VMEM((D, D), bf16),
        pltpu.VMEM((D, D), bf16),
        pltpu.VMEM((D, D), bf16),
        pltpu.VMEM((D, F), bf16),
        pltpu.VMEM((F, D), bf16),
        pltpu.VMEM((1, H), bf16),
        pltpu.VMEM((S, D), f32),
        pltpu.VMEM((S, D), f32),
        pltpu.VMEM((S, D), bf16),
        pltpu.VMEM((L, D), bf16),
        pltpu.VMEM((S + 2 * HALO, D), f32),
        pltpu.VMEM((L, HC), bf16),
        pltpu.VMEM((L, HC), bf16),
        pltpu.VMEM((HC, L), bf16),
        pltpu.VMEM((HC, L), bf16),
        pltpu.VMEM((HC, L), bf16),
        pltpu.VMEM((2, S, HC), bf16),
        pltpu.VMEM((NG, MZR, 128), f32),
        pltpu.VMEM((MZR, 128), f32),
        pltpu.VMEM((128, 128), f32),
        pltpu.VMEM((2, H // 2, 128), f32),
        pltpu.VMEM((8, 128), jnp.uint32),
        pltpu.SMEM((1,), jnp.int32),
        pltpu.SemaphoreType.DMA((13,)),
        pltpu.SemaphoreType.DMA((S // TB,)),
        pltpu.SemaphoreType.DMA((S // TB,)),
    ]
    out = pl.pallas_call(
        _kernel,
        out_shape=jax.ShapeDtypeStruct((S, D), bf16),
        in_specs=[any_spec] * 10,
        out_specs=any_spec,
        scratch_shapes=scratch,
        compiler_params=pltpu.CompilerParams(vmem_limit_bytes=112 * 1024 * 1024),
    )(x, A_wq, A_wk, A_wv, A_wo, beta, B_w1, B_w2, B_w3, B_w4)
    return out.reshape(1, S, D)
```

```python
import functools
import math

import jax
import jax.numpy as jnp
from jax import lax
import jax.experimental.pallas as pl
import jax.experimental.pallas.tpu as pltpu

f32 = jnp.float32
bf16 = jnp.bfloat16

S = 2048
D = 1024
F = 3584
H = 32
DH = 32
L = 512
NSEG = S // L
NG = D // 128
HC = D // 2
GH = HC // 128
TB = 256
FC = 512
HALO = 8
MZR = 144
EPS = 1e-5
NEG = -1e30
QSCALE = (DH ** -0.5) * math.log2(math.e)
GELU_C0 = math.sqrt(2.0 / math.pi)
GELU_C1 = GELU_C0 * 0.044715
ATT_LAG = 2
LN_LEAD = 2
W1_DUE = 4
W1_LN = (3, 3, 4, 4, 5, 5, 6, 6, 7, 7, 8)
LNC = 16
YR = 176
SCHEDULE = (
    (-1, "ln", "y", (0, 1, 2, 3), 0), (-1, "k", 0, 0), (-1, "qv", 0, 0), (-1, "qv", 0, 1), (0, "qv", 0, 2),
    (0, "ret", 0, 0), (2, "k", 0, 1), (3, "qv", 0, 3), (3, "ln", "y", (4,), 4), (4, "ln", "y", (5,), 5),
    (5, "ret", 0, 1), (5, "k", 1, 0), (6, "ln", "y", (6,), 7), (7, "ln", "y", (7,), 8), (7, "qv", 1, 0),
    (8, "qv", 1, 1), (9, "ln", "y", (8,), 10), (10, "ln", "y", (9,), 11), (11, "ret", 1, 0), (11, "qv", 1, 2),
    (11, "ln", "y", (10,), 12), (12, "k", 1, 1), (13, "ln", "y", (11,), 14), (14, "qv", 1, 3),
    (14, "k", 2, 0), (16, "ret", 1, 1), (16, "ln", "y", (13,), 17), (16, "wo", 0, 0),
    (16, "ln", "y", (12,), 17), (18, "ln", "y", (14,), 19), (19, "qv", 2, 0), (19, "qv", 2, 1),
    (19, "ln", "y", (15,), 20), (19, "ln", "x", (1,), 20), (20, "ret", 2, 0), (21, "qv", 2, 2),
    (21, "ln", "x", (0,), 22), (22, "k", 2, 1), (23, "qv", 2, 3), (23, "ln", "x", (2,), 24), (23, "k", 3, 0),
    (24, "ln", "x", (3,), 25), (25, "ln", "x", (4,), 26), (26, "wo", 0, 1), (26, "ln", "x", (5,), 27),
    (27, "ret", 2, 1), (27, "qv", 3, 0), (27, "ln", "x", (6,), 28), (28, "ln", "x", (7,), 29),
    (29, "qv", 3, 1), (29, "ln", "x", (8,), 30), (30, "ln", "x", (9,), 31), (31, "qv", 3, 2),
    (31, "ln", "x", (11,), 32), (32, "k", 3, 1), (32, "ret", 3, 0), (33, "ln", "x", (10,), 34),
    (33, "ln", "x", (12,), 34), (34, "qv", 3, 3), (34, "wo", 0, 2), (34, "ln", "x", (13,), 35),
    (35, "wo", 0, 3), (36, "ln", "x", (14,), 37), (36, "ln", "x", (15,), 37), (36, "wo", 1, 0),
    (36, "mem", 0), (36, "mem", 1), (37, "ret", 3, 1), (40, "mem", 3), (41, "wo", 1, 1), (41, "mem", 2),
    (42, "wo", 1, 2), (42, "wo", 1, 3),
)


def _dot(a, b):
    return jnp.dot(a, b, preferred_element_type=f32)


def _dot_nt(a, b):
    return lax.dot_general(a, b, (((1,), (1,)), ((), ())), preferred_element_type=f32)


def _ln(x):
    m = jnp.mean(x, axis=-1, keepdims=True)
    xc = x - m
    v = jnp.mean(xc * xc, axis=-1, keepdims=True)
    return xc * lax.rsqrt(v + EPS)


def _ln_chunks(mean, load, zero, post, prev=None, sel=None):
    outs = []
    for i in sel or range(mean.shape[0] // LNC):
        m = mean[LNC * i:LNC * i + LNC]
        if prev is not None:
            m = pltpu.bitcast(pltpu.bitcast(m, jnp.int32) | (pltpu.bitcast(prev, jnp.int32) & zero), f32)
        xc = load(i) - m
        prev = lax.rsqrt(jnp.mean(xc * xc, axis=-1, keepdims=True) + EPS)
        outs.append(post(i, xc * prev))
    return outs


def _rowmean(x):
    return jnp.mean(x, axis=-1, keepdims=True)


def _gelu(x):
    t = jnp.tanh(x * (GELU_C0 + GELU_C1 * (x * x)))
    hx = 0.5 * x
    return hx + hx * t


def _phi(t):
    return jnp.where(t > 0, t + 1.0, jnp.exp(t))


def _fold(x, op):
    parts = [x[8 * i:8 * i + 8] for i in range(x.shape[0] // 8)]
    while len(parts) > 1:
        parts = [op(parts[i], parts[i + 1]) for i in range(0, len(parts), 2)]
    return parts[0]


def _after(x, deps, never):
    d = functools.reduce(jnp.bitwise_or, [pltpu.bitcast(v, jnp.uint32) for v in deps])
    bits = pltpu.bitcast(x, jnp.uint32)
    top = jnp.concatenate([jnp.where(never, d, bits[0:8, 0:128]), bits[0:8, 128:]], axis=1)
    return pltpu.bitcast(jnp.concatenate([top, bits[8:]], axis=0), x.dtype)


def _paced(x, pace, never):
    bits = pltpu.bitcast(x, jnp.uint32)
    return pltpu.bitcast(jnp.where(never, pltpu.bitcast(pace[0:bits.shape[0]], jnp.uint32), bits), x.dtype)


def _attention(k_ref, qt_ref, vt_ref, mem, run, gate_ref, mask_ref, o_ref, hooks, ties, never):
    steps = [(g, j, t) for g in range(GH) for j in range(4) for t in range(j + 1)]
    scores, outs = {}, {}
    drained = []

    lane = lax.broadcasted_iota(jnp.int32, (1, 128), 1)
    late = [lane < 64, lane >= 64]

    def keep(x, h):
        bits = pltpu.bitcast(x, jnp.uint32)
        return pltpu.bitcast(jnp.where(late[h % 2], bits, jnp.uint32(0)), bf16)

    def pad(x, r):
        parts = [jnp.zeros((r, 128), bf16), x, jnp.zeros((128 - r - x.shape[0], 128), bf16)]
        return jnp.concatenate([v for v in parts if v.shape[0]], axis=0)

    def do_qk(n):
        g, j, t = steps[n]
        gs = slice(128 * g, 128 * g + 128)
        q = [qt_ref[128 * g + 32 * h:128 * g + 32 * h + 32, 128 * j:128 * j + 128] for h in range(4)]
        w = jnp.concatenate([pad(q[h], 32 * h) for h in range(4)], axis=1)
        if t < j:
            scores[n] = (_dot(k_ref[128 * t:128 * t + 128, gs], w), None)
            return
        w2 = [pad(jnp.concatenate([keep(q[h], h), keep(q[h + 1], h + 1)], axis=0), 32 * h) for h in (0, 2)]
        s1 = _dot(k_ref[128 * t:128 * t + 64, gs], w)
        s2 = [jnp.concatenate([_dot(k_ref[128 * t + r:128 * t + r + 32, gs], v) for r in (64, 96)], axis=0)
              for v in w2]
        scores[n] = (s1, jnp.concatenate(s2, axis=1))

    def do_sm(n):
        g, j, t = steps[n]
        st, st2 = scores.pop(n)
        cur, cur2 = [], []
        for h in range(4):
            s = st[:, 128 * h:128 * h + 128]
            if t == j:
                s = s + mask_ref[h % 2]
            mx = _fold(s, jnp.maximum)
            if t == j:
                if h % 2 == 0:
                    s2 = st2[:, 64 * h:64 * h + 128] + mask_ref[2]
                    cur2.append((s2, _fold(s2, jnp.maximum)))
                mx = jnp.where(late[h % 2], jnp.maximum(mx, cur2[-1][1]), mx)
            m = jnp.max(mx, axis=0, keepdims=True)
            if t > 0:
                m = jnp.maximum(m, run[h][0])
            if h == 0 and n in ties:
                m = jnp.where(never, functools.reduce(jnp.add, ties[n]), m)
            cur.append((s, m))
        res = []
        for h in range(4):
            s, m = cur[h]
            r0 = 128 * g + 32 * h
            p = jnp.exp2(s - m)
            sm = _fold(p, jnp.add)
            pb = p.astype(bf16)
            if t == j:
                if h % 2 == 0:
                    p2 = jnp.exp2(cur2[h // 2][0] - jnp.where(late[0], m, cur[h + 1][1]))
                    sm2, pb2 = _fold(p2, jnp.add), p2.astype(bf16)
                sm = jnp.where(late[h % 2], sm + sm2, sm)
                pb = jnp.concatenate([pb, keep(pb2, h)], axis=0)
            o = _dot(vt_ref[r0:r0 + 32, 128 * t:128 * t + 128], pb)
            res.append((m, o, sm))
        for h in range(4):
            m, o, sm = res[h]
            if t > 0:
                a = jnp.exp2(run[h][0] - m)
                o = run[h][1] * a + o
                sm = run[h][2] * a + sm
            run[h] = (m, o, sm)
            if t == j:
                gate = gate_ref[4 * g + h:4 * g + h + 1, :]
                if drained:
                    sm = jnp.where(never, drained.pop(), sm)
                l = jnp.sum(sm, axis=0, keepdims=True)
                r = mem[g, j // 2][:, 128 * (j % 2):128 * (j % 2) + 128]
                den = r[128 + h:129 + h] + 1e-6
                outs[h] = r[32 * h:32 * h + 32] * (gate / den) + o * ((1.0 - gate) / l)
        if t == j:
            ot = jnp.concatenate([outs[h] for h in range(4)], axis=0)
            ob = pltpu.bitcast(ot.T.astype(bf16), jnp.uint32)
            even = (lane // DH) % 2 == 0
            ob = jnp.concatenate([jnp.where(even, ob[32:64], ob[0:32]), jnp.where(even, ob[0:32], ob[32:64])], axis=0)
            o_ref[128 * j:128 * j + 128, 128 * g:128 * g + 128] = pltpu.bitcast(ob, bf16)
            drained.append(pltpu.bitcast(ob[56:64], f32))

    n_steps = len(steps)
    for n in range(n_steps + ATT_LAG):
        if n < n_steps:
            do_qk(n)
        for p in hooks.get(n, []):
            p()
        if n >= ATT_LAG:
            do_sm(n - ATT_LAG)
    for p in hooks.get(n_steps + ATT_LAG, []):
        p()


def _kernel(x_hbm, wq_hbm, wk_hbm, wv_hbm, wo_hbm, beta_hbm, w1_hbm, w2_hbm, w3_hbm, w4_hbm,
            out_hbm,
            xio, wqv_s, wk_v, wqvt, wo_v, w1_v, w2_v, w3_v, w4_v, beta_v,
            x_ref, y_ref, xn_ref, xc_ref, xa_ref, h_ref,
            k_ref, pk_ref, qt_ref, pqt_ref, vt_ref, o_ref,
            mz_ref, mzmask_ref, mask_ref, gate_ref, zs_ref,
            sem_in, sem_x, sem_out):
    def cp(src, dst, i):
        return pltpu.make_async_copy(src, dst, sem_in.at[i])

    def x_cp(t):
        r0 = t * TB if isinstance(t, int) else pl.multiple_of(t * TB, TB)
        return pltpu.make_async_copy(x_hbm.at[pl.ds(r0, TB)], xio.at[pl.ds(r0, TB)], sem_x.at[t])

    def out_cp(t):
        r0 = t * TB if isinstance(t, int) else pl.multiple_of(t * TB, TB)
        return pltpu.make_async_copy(xio.at[pl.ds(r0, TB)], out_hbm.at[pl.ds(r0, TB)], sem_out.at[t])

    wqv_cp = [cp(w.at[:, pl.ds(HC * a, HC)], wqv_s.at[2 * a + i], 2 * a + i)
              for a in range(2) for i, w in enumerate((wq_hbm, wv_hbm))]
    wk_cp = [cp(wk_hbm.at[:, pl.ds(HC * a, HC)], wk_v.at[a], 4 + a) for a in range(2)]
    wo_cp = [cp(wo_hbm.at[pl.ds(HC * a, HC)], wo_v.at[a], 12 + a) for a in range(2)]
    beta_cp = cp(beta_hbm, beta_v, 6)
    w1_cp = cp(w1_hbm, w1_v, 8)
    w2_cp = cp(w2_hbm, w2_v, 9)
    w3_cp = cp(w3_hbm, w3_v, 10)
    w4_cp = cp(w4_hbm, w4_v, 11)

    for c in [beta_cp, x_cp(0), x_cp(1), wqv_cp[0]]:
        c.start()

    kk = lax.broadcasted_iota(jnp.int32, (64, 128), 0)
    qq = lax.broadcasted_iota(jnp.int32, (64, 128), 1)
    for i, q_pos in enumerate(((qq + 64) % 128, qq, qq % 64)):
        mask_ref[i] = jnp.where(kk <= q_pos, 0.0, NEG).astype(f32)
    rr = lax.broadcasted_iota(jnp.int32, (MZR, 128), 0)
    cc = lax.broadcasted_iota(jnp.int32, (MZR, 128), 1) // DH
    row_head = jnp.where(rr < 128, rr // DH, rr - 128)
    mzmask_ref[...] = jnp.where(row_head == cc, 1.0, 0.0).astype(f32)
    zs_ref[0] = jnp.int32(0)
    h_ref[0:HALO, :] = jnp.zeros((HALO, D), f32)
    h_ref[HALO + S:HALO + S + HALO, :] = jnp.zeros((HALO, D), f32)

    beta_cp.wait()
    eye = (lax.broadcasted_iota(jnp.int32, (H, H), 0) == lax.broadcasted_iota(jnp.int32, (H, H), 1))
    beta_rows = jnp.broadcast_to(beta_v[...].astype(f32), (H, H))
    beta_col = jnp.sum(jnp.where(eye, beta_rows, 0.0), axis=1, keepdims=True)
    gates = jnp.broadcast_to(jax.nn.sigmoid(beta_col), (H, 128))
    gate_ref[0] = gates[0:H // 2]
    gate_ref[1] = gates[H // 2:H]

    def loop(n, fn, name):
        def body(i, c):
            with jax.named_scope(name):
                fn(i)
            return c

        lax.fori_loop(0, n, body, 0)

    def never():
        return zs_ref[0] != 0

    def chunk(r0, i):
        return pl.ds(pl.multiple_of(r0 + LNC * i, LNC), LNC)

    def norm_rows(r0, n, dsts):
        def load(i):
            return xio[chunk(r0, i), :].astype(f32)

        def post(i, y):
            for dst in dsts:
                dst[chunk(r0, i), :] = y.astype(bf16)
            return [y[r:r + 1, 0:128] for r in range(0, LNC, 8)]

        mean = _rowmean(xio[pl.ds(pl.multiple_of(r0, LNC), n), :].astype(f32))
        return functools.partial(_ln_chunks, mean, load, zs_ref[0], post)

    def mixer_norm(r0, n):
        def post(i, y):
            y_ref[chunk(r0, i), :] = y
            yn = _ln(y)
            xn_ref[chunk(S + r0, i), :] = yn.astype(bf16)
            return [yn[r:r + 1, 0:128] for r in range(0, LNC, 8)]

        mean = _rowmean(x_ref[pl.ds(pl.multiple_of(r0, LNC), n), :])
        return functools.partial(_ln_chunks, mean, lambda i: x_ref[chunk(r0, i), :], zs_ref[0], post)

    def pt_body(layer, u):
        s = u // 2
        a = u % 2

        @pl.when(jnp.logical_and(layer == 0, u < 2))
        def _():
            def tr(i):
                src = wqv_s.at[2 * u + i]
                pltpu.make_async_copy(src, src, sem_in.at[2 * u + i]).wait()
                wt = src[...].T
                for g in range(GH):
                    wqvt[u, g, pl.ds(pl.multiple_of(128 * i, 128), 128), :] = wt[128 * g:128 * g + 128]

            loop(2, tr, "transpose")
            pltpu.make_async_copy(wk_v.at[u], wk_v.at[u], sem_in.at[4 + u]).wait()
            pltpu.make_async_copy(wo_v.at[u], wo_v.at[u], sem_in.at[12 + u]).wait()

            @pl.when(u == 0)
            def _():
                for c in [wqv_cp[2], wqv_cp[3], wk_cp[1], wo_cp[1], x_cp(3)]:
                    c.start()

            @pl.when(u == 1)
            def _():
                for c in [x_cp(t) for t in range(4, S // TB)] + [w1_cp]:
                    c.start()

        @pl.when(jnp.logical_and(layer == 0, u < S // TB - 2))
        def _():
            x_cp(u + 2).wait()

            @pl.when(u == 2)
            def _():
                w2_cp.start()
                w3_cp.start()

            @pl.when(u == 4)
            def _():
                w4_cp.start()

        r0 = pl.multiple_of(s * L, L)
        g0 = GH * a
        mem, run, ties = {}, {}, {}

        norms = {"x": norm_rows(((s + 1) % NSEG) * L + a * TB, TB, [xn_ref]),
                 "y": mixer_norm(((s + NSEG - 1) % NSEG) * L + a * TB, TB)}

        def norm(kind, sel, due):
            after = jnp.concatenate([run[0][2][:, 0:1]] * (LNC // 8), axis=0) if run else None
            for i, v in enumerate(norms[kind](after, sel)):
                ties.setdefault(due + i, []).extend(v)

        def qv_proj(g, c):
            gs, cs = slice(128 * g, 128 * g + 128), slice(128 * c, 128 * c + 128)
            r = _dot_nt(wqvt[a, g], xc_ref[cs, :])
            q = jnp.concatenate([r[32 * h:32 * h + 32] if h % 2 else pltpu.roll(r[32 * h:32 * h + 32], 64, 1)
                                 for h in range(4)], axis=0)
            qt_ref[gs, cs] = (q * QSCALE).astype(bf16)
            pqt_ref[gs, cs] = _phi(q).astype(bf16)
            vt_ref[gs, cs] = r[128:256].astype(bf16)

        def k_proj(g, c):
            gs, rs = slice(128 * g, 128 * g + 128), slice(256 * c, 256 * c + 256)
            kf = _dot(xc_ref[rs, :], wk_v[a, :, gs])
            k_ref[rs, gs] = kf.astype(bf16)
            pk_ref[rs, gs] = _phi(kf).astype(bf16)

        def retrieve(g, c):
            mzb = mz_ref[g0 + g].astype(bf16)
            mem[g, c] = jnp.concatenate([
                jnp.concatenate([_dot(mzb[rs], pqt_ref[128 * g:128 * g + 128, 128 * j:128 * j + 128])
                                 for rs in (slice(0, r), slice(r, MZR))], axis=0)
                for j, r in ((2 * c, 64 + 16 * c), (2 * c + 1, 64 + 16 * c))], axis=1)

        def mem_update(g):
            ones = jnp.ones((MZR - 128, L), bf16)
            lhs = jnp.concatenate([vt_ref[128 * g:128 * g + 128, :], ones], axis=0)
            upd = _dot(lhs, pk_ref[:, 128 * g:128 * g + 128])
            mz_ref[g0 + g] = jnp.where(s == NSEG - 1, 0.0, mz_ref[g0 + g] + upd * mzmask_ref[...])

        def out_proj(part, j):
            rows = pl.ds(pl.multiple_of(r0 + 128 * j, 128), 128)
            rs, ks = slice(128 * j, 128 * j + 128), slice(256 * part, 256 * part + 256)
            upd = _dot(o_ref[rs, ks], wo_v[a, ks, :])
            if part == 0:
                xa_ref[rs, :] = upd
            else:
                base = jnp.where(a == 0, xio[rows, :].astype(f32), x_ref[rows, :])
                x_ref[rows, :] = base + xa_ref[rs, :] + upd
                nxt = (u + 1) // 2
                xc_ref[rs, :] = _paced(xn_ref[pl.ds(pl.multiple_of(nxt * L + 128 * j, 128), 128), :], upd, never())

        work = {"qv": qv_proj, "k": k_proj, "ret": retrieve, "mem": mem_update, "wo": out_proj,
                "ln": norm}
        hooks = {}
        for n, kind, *args in SCHEDULE:
            hooks.setdefault(n, []).append(functools.partial(work[kind], *args))
        for p in hooks.pop(-1):
            p()
        _attention(k_ref, qt_ref, vt_ref, mem, run, gate_ref.at[a], mask_ref, o_ref, hooks, ties,
                   never())

    def w1_body(s):
        r0 = pl.multiple_of(s * L, L)
        norm = mixer_norm(S - L + jnp.minimum(s * YR, L - YR), YR)
        src = [r0 + S + TB, jnp.minimum(r0 + L, S - L) + S]
        done = {}
        for p in range(2 * D // 128):
            a, c = divmod(p, D // 128)
            lhs = xc_ref[TB * a:TB * a + TB, :]
            r = _dot(_after(lhs, done[p], never()) if p in done else lhs, w1_v[:, 128 * c:128 * c + 128])
            h_ref[pl.ds(pl.multiple_of(r0 + TB * a + HALO, 8), TB), 128 * c:128 * c + 128] = _gelu(r)
            if c // 4 == a:
                cs = slice(256 * (c % 4), 256 * (c % 4) + 256)
                xc_ref[TB - TB * a:L - TB * a, cs] = _paced(
                    xn_ref[pl.ds(pl.multiple_of(src[a], TB), TB), cs],
                    jnp.concatenate([r[0:128], r[128:256]], axis=1), never())
            sel = [i for i, n in enumerate(W1_LN) if n == p]
            if sel:
                done[p + W1_DUE] = sum(norm(r[0:LNC, 0:1], sel), [])

    def mix_body(layer, t):
        r0 = pl.multiple_of(t * TB, TB)
        half = TB // 2
        c4 = D // 4
        hs = []
        for a in range(2):
            win = h_ref[pl.ds(pl.multiple_of(r0 + half * a, half), half + 2 * HALO), :]
            hs.append(jnp.concatenate([
                pltpu.roll(win[:, c4 * i:c4 * i + c4], d % (half + 2 * HALO), 0)[HALO:HALO + half].astype(bf16)
                for i, d in enumerate((1, -1, 2, -2))], axis=1))

        def norm(a, upd, gates):
            ra = pl.multiple_of(r0 + half * a, half)
            x1 = y_ref[pl.ds(ra, half), :] + jnp.concatenate(upd, axis=1)
            xa_ref[half * a:half * a + half, :] = x1
            mean = _rowmean(x1)
            out = []
            for i in range(half // LNC):
                gate = gates[i - LN_LEAD][0:LNC, 0:1] if i >= LN_LEAD else None
                out += _ln_chunks(mean, lambda i: xa_ref[pl.ds(half * a + LNC * i, LNC), :], zs_ref[0],
                                  lambda i, y: y.astype(bf16), gate, (i,))
            return jnp.concatenate(out, axis=0)

        def up(lhs, c):
            return _gelu(_dot(lhs, w3_v[:, FC * c:FC * c + FC]))

        cols = range(0, D, 128)
        upd0 = [_dot(_after(hs[0], [hs[1][r:r + 16, c - 128:c] for r in range(0, half, 16)], never()) if c else hs[0], w2_v[:, c:c + 128])
                for c in cols]
        upd1 = [_dot(hs[1], w2_v[:, c:c + 128]) for c in cols]
        x1n = [norm(0, upd0, upd1)]
        pre = [_dot(x1n[0], w3_v[:, c:c + 128]) for c in range(0, 2 * FC, 128)]
        x1n.append(norm(1, upd1, pre))
        pre = _gelu(jnp.concatenate(pre, axis=1))
        nch = F // FC
        x1n_full = jnp.concatenate(x1n, axis=0)
        hid = {c: jnp.concatenate([pre[:, FC * c:FC * c + FC], up(x1n[1], c)], axis=0).astype(bf16)
               for c in range(2)}
        acc = x_ref[pl.ds(r0, TB), :] + xa_ref[0:TB, :]
        xr = (nch - 2) * LNC
        next_norm = norm_rows(jnp.clip((t - 1) * xr, 0, L - xr), xr, [xn_ref, xc_ref])
        for c in range(nch):
            acc = acc + _dot(hid.pop(c), w4_v[FC * c:FC * c + FC, :])
            if c + 2 < nch:
                act = up(x1n_full, c + 2)
                hid[c + 2] = _after(act.astype(bf16), next_norm(act[0:LNC, 0:1], [c])[0], never())
        xio[pl.ds(r0, TB), :] = acc.astype(bf16)

        @pl.when(layer == 1)
        def _():
            out_cp(t).start()

    def norm0(i):
        x_ref[pl.ds(pl.multiple_of(S - L + i * TB, TB), TB), :] = jnp.zeros((TB, D), f32)
        x_cp(i).wait()

        @pl.when(i == 0)
        def _():
            wqv_cp[1].start()

        @pl.when(i == 1)
        def _():
            wk_cp[0].start()
            wo_cp[0].start()
            x_cp(2).start()

        rows = pl.ds(pl.multiple_of(i * TB, TB), TB)
        xn = _ln(xio[rows, :].astype(f32)).astype(bf16)
        xn_ref[rows, :] = xn
        xc_ref[rows, :] = xn

    mz_ref[...] = jnp.zeros(mz_ref.shape, f32)
    loop(L // TB, norm0, "norm0")

    def layer_body(layer):
        loop(2 * NSEG, lambda u: pt_body(layer, u), "pt")

        @pl.when(layer == 0)
        def _():
            w1_cp.wait()

        loop(NSEG, w1_body, "w1")

        @pl.when(layer == 0)
        def _():
            w2_cp.wait()
            w3_cp.wait()
            w4_cp.wait()

        loop(S // TB, lambda t: mix_body(layer, t), "mix")

    loop(2, layer_body, "layer")
    for t in range(S // TB):
        out_cp(t).wait()


@jax.jit
def pallas_interleave_layers__memory_aug_infini_attn__mixer_s_mlp__prompt_kernel(
    A_x: jax.Array,
    A_wq: jax.Array,
    A_wk: jax.Array,
    A_wv: jax.Array,
    A_wo: jax.Array,
    A_beta: jax.Array,
    B_x: jax.Array,
    B_w1: jax.Array,
    B_w2: jax.Array,
    B_w3: jax.Array,
    B_w4: jax.Array,
):
    del B_x
    x = A_x.reshape(S, D)
    beta = A_beta.reshape(1, H)
    any_spec = pl.BlockSpec(memory_space=pl.ANY)
    scratch = [
        pltpu.VMEM((S, D), bf16),
        pltpu.VMEM((4, D, HC), bf16),
        pltpu.VMEM((2, D, HC), bf16),
        pltpu.VMEM((2, GH, 256, D), bf16),
        pltpu.VMEM((2, HC, D), bf16),
        pltpu.VMEM((D, D), bf16),
        pltpu.VMEM((D, D), bf16),
        pltpu.VMEM((D, F), bf16),
        pltpu.VMEM((F, D), bf16),
        pltpu.VMEM((1, H), bf16),
        pltpu.VMEM((S, D), f32),
        pltpu.VMEM((S, D), f32),
        pltpu.VMEM((2 * S, D), bf16),
        pltpu.VMEM((L, D), bf16),
        pltpu.VMEM((L, D), f32),
        pltpu.VMEM((S + 2 * HALO, D), f32),
        pltpu.VMEM((L, HC), bf16),
        pltpu.VMEM((L, HC), bf16),
        pltpu.VMEM((HC, L), bf16),
        pltpu.VMEM((HC, L), bf16),
        pltpu.VMEM((HC, L), bf16),
        pltpu.VMEM((L, HC), bf16),
        pltpu.VMEM((NG, MZR, 128), f32),
        pltpu.VMEM((MZR, 128), f32),
        pltpu.VMEM((3, 64, 128), f32),
        pltpu.VMEM((2, H // 2, 128), f32),
        pltpu.SMEM((1,), jnp.int32),
        pltpu.SemaphoreType.DMA((14,)),
        pltpu.SemaphoreType.DMA((S // TB,)),
        pltpu.SemaphoreType.DMA((S // TB,)),
    ]
    out = pl.pallas_call(
        _kernel,
        out_shape=jax.ShapeDtypeStruct((S, D), bf16),
        in_specs=[any_spec] * 10,
        out_specs=any_spec,
        scratch_shapes=scratch,
        compiler_params=pltpu.CompilerParams(vmem_limit_bytes=112 * 1024 * 1024),
    )(x, A_wq, A_wk, A_wv, A_wo, beta, B_w1, B_w2, B_w3, B_w4)
    return out.reshape(1, S, D)
```

```python
import functools
import math

import jax
import jax.numpy as jnp
from jax import lax
import jax.experimental.pallas as pl
import jax.experimental.pallas.tpu as pltpu

f32 = jnp.float32
bf16 = jnp.bfloat16

S = 2048
D = 1024
F = 3584
H = 32
DH = 32
L = 512
NSEG = S // L
NG = D // 128
HC = D // 2
GH = HC // 128
TB = 256
FC = 512
MZR = 144
EPS = 1e-5
NEG = -1e30
QSCALE = (DH ** -0.5) * math.log2(math.e)
GELU_C0 = math.sqrt(2.0 / math.pi)
GELU_C1 = GELU_C0 * 0.044715
ATT_LAG = 2
LN_LEAD = 2
MIX_LN = (0, 0, 1, 1, 2, 2, 3, 3, 4, 4, 5, 5, 5, 6, 6, 6)
LNC = 16
TR_MXU = (0, 3, 6)
W1_ORDER = (512, 640, 768, 896, 0, 128, 256, 384)
YR = 48
SCHEDULE = (
    (-1, "ln", "y", (0, 1, 2), 0), (-1, "k", 0, 0), (-1, "qv", 0, 0), (-1, "qv", 0, 1), (0, "qv", 0, 2),
    (0, "ret", 0, 0), (2, "k", 0, 1), (4, "qv", 0, 3), (5, "ret", 0, 1), (5, "k", 1, 0), (7, "qv", 1, 0),
    (8, "qv", 1, 1), (11, "ret", 1, 0), (11, "qv", 1, 2), (11, "k", 1, 1), (12, "ln", "x", (0,), 13),
    (13, "ln", "x", (1,), 14), (14, "qv", 1, 3), (14, "k", 2, 0), (14, "ln", "x", (2,), 15),
    (16, "ret", 1, 1), (16, "wo", 0, 0), (16, "ln", "x", (3,), 17), (18, "ln", "x", (4,), 19),
    (19, "qv", 2, 0), (19, "qv", 2, 1), (20, "ret", 2, 0), (21, "qv", 2, 3), (21, "qv", 2, 2),
    (21, "ln", "x", (6,), 22), (22, "k", 2, 1), (22, "ln", "x", (5,), 23), (23, "k", 3, 0),
    (25, "ln", "x", (7,), 26), (25, "ln", "x", (9,), 26), (25, "ln", "x", (8,), 26), (26, "wo", 0, 1),
    (27, "ret", 2, 1), (27, "qv", 3, 0), (27, "ln", "x", (10,), 28), (28, "ln", "x", (11,), 29),
    (29, "qv", 3, 1), (30, "qv", 3, 2), (30, "ln", "x", (12,), 31), (31, "ln", "x", (13,), 32),
    (32, "k", 3, 1), (32, "ret", 3, 0), (33, "ln", "x", (14,), 34), (34, "qv", 3, 3), (34, "wo", 0, 2),
    (34, "mem", 0), (34, "ln", "x", (15,), 35), (35, "wo", 0, 3), (36, "wo", 1, 0), (36, "mem", 1),
    (37, "ret", 3, 1), (40, "mem", 3), (41, "wo", 1, 1), (41, "mem", 2), (42, "wo", 1, 2), (42, "wo", 1, 3),
)


def _dot(a, b):
    return jnp.dot(a, b, preferred_element_type=f32)


def _dot_nt(a, b):
    return lax.dot_general(a, b, (((1,), (1,)), ((), ())), preferred_element_type=f32)


def _ln(x):
    m = jnp.mean(x, axis=-1, keepdims=True)
    xc = x - m
    v = jnp.mean(xc * xc, axis=-1, keepdims=True)
    return xc * lax.rsqrt(v + EPS)


def _ln_chunks(mean, load, zero, post, prev=None, sel=None):
    outs = []
    for i in sel or range(mean.shape[0] // LNC):
        m = mean[LNC * i:LNC * i + LNC]
        if prev is not None:
            m = pltpu.bitcast(pltpu.bitcast(m, jnp.int32) | (pltpu.bitcast(prev, jnp.int32) & zero), f32)
        xc = load(i) - m
        prev = lax.rsqrt(jnp.mean(xc * xc, axis=-1, keepdims=True) + EPS)
        outs.append(post(i, xc * prev))
    return outs


def _rowmean(x):
    return jnp.mean(x, axis=-1, keepdims=True)


def _gelu(x):
    t = jnp.tanh(x * (GELU_C0 + GELU_C1 * (x * x)))
    hx = 0.5 * x
    return hx + hx * t


def _phi(t):
    return jnp.where(t > 0, t + 1.0, jnp.exp(t))


def _fold(x, op):
    parts = [x[8 * i:8 * i + 8] for i in range(x.shape[0] // 8)]
    while len(parts) > 1:
        parts = [op(parts[i], parts[i + 1]) for i in range(0, len(parts), 2)]
    return parts[0]


def _after(x, deps, never):
    d = functools.reduce(jnp.bitwise_or, [pltpu.bitcast(v, jnp.uint32) for v in deps])
    bits = pltpu.bitcast(x, jnp.uint32)
    top = jnp.concatenate([jnp.where(never, d, bits[0:8, 0:128]), bits[0:8, 128:]], axis=1)
    return pltpu.bitcast(jnp.concatenate([top, bits[8:]], axis=0), x.dtype)


def _paced(x, pace, never):
    bits = pltpu.bitcast(x, jnp.uint32)
    return pltpu.bitcast(jnp.where(never, pltpu.bitcast(pace[0:bits.shape[0]], jnp.uint32), bits), x.dtype)


def _attention(k_ref, qt_ref, vt_ref, mem, run, gate_ref, mask_ref, o_ref, hooks, ties, never):
    steps = [(g, j, t) for g in range(GH) for j in range(4) for t in range(j + 1)]
    scores, outs = {}, {}
    drained = []

    lane = lax.broadcasted_iota(jnp.int32, (1, 128), 1)
    late = [lane < 64, lane >= 64]

    def keep(x, h):
        bits = pltpu.bitcast(x, jnp.uint32)
        return pltpu.bitcast(jnp.where(late[h % 2], bits, jnp.uint32(0)), bf16)

    def pad(x, r):
        parts = [jnp.zeros((r, 128), bf16), x, jnp.zeros((128 - r - x.shape[0], 128), bf16)]
        return jnp.concatenate([v for v in parts if v.shape[0]], axis=0)

    def do_qk(n):
        g, j, t = steps[n]
        gs = slice(128 * g, 128 * g + 128)
        q = [qt_ref[128 * g + 32 * h:128 * g + 32 * h + 32, 128 * j:128 * j + 128] for h in range(4)]
        w = jnp.concatenate([pad(q[h], 32 * h) for h in range(4)], axis=1)
        if t < j:
            scores[n] = (_dot(k_ref[128 * t:128 * t + 128, gs], w), None)
            return
        w2 = [pad(jnp.concatenate([keep(q[h], h), keep(q[h + 1], h + 1)], axis=0), 32 * h) for h in (0, 2)]
        s1 = _dot(k_ref[128 * t:128 * t + 64, gs], w)
        s2 = [jnp.concatenate([_dot(k_ref[128 * t + r:128 * t + r + 32, gs], v) for r in (64, 96)], axis=0)
              for v in w2]
        scores[n] = (s1, jnp.concatenate(s2, axis=1))

    def do_sm(n):
        g, j, t = steps[n]
        st, st2 = scores.pop(n)
        cur, cur2 = [], []
        for h in range(4):
            s = st[:, 128 * h:128 * h + 128]
            if t == j:
                s = s + mask_ref[h % 2]
            mx = _fold(s, jnp.maximum)
            if t == j:
                if h % 2 == 0:
                    s2 = st2[:, 64 * h:64 * h + 128] + mask_ref[2]
                    cur2.append((s2, _fold(s2, jnp.maximum)))
                mx = jnp.where(late[h % 2], jnp.maximum(mx, cur2[-1][1]), mx)
            m = jnp.max(mx, axis=0, keepdims=True)
            if t > 0:
                m = jnp.maximum(m, run[h][0])
            if h == 0 and n in ties:
                m = jnp.where(never, functools.reduce(jnp.add, ties[n]), m)
            cur.append((s, m))
        res = []
        for h in range(4):
            s, m = cur[h]
            r0 = 128 * g + 32 * h
            p = jnp.exp2(s - m)
            sm = _fold(p, jnp.add)
            pb = p.astype(bf16)
            if t == j:
                if h % 2 == 0:
                    p2 = jnp.exp2(cur2[h // 2][0] - jnp.where(late[0], m, cur[h + 1][1]))
                    sm2, pb2 = _fold(p2, jnp.add), p2.astype(bf16)
                sm = jnp.where(late[h % 2], sm + sm2, sm)
                pb = jnp.concatenate([pb, keep(pb2, h)], axis=0)
            o = _dot(vt_ref[r0:r0 + 32, 128 * t:128 * t + 128], pb)
            res.append((m, o, sm))
        for h in range(4):
            m, o, sm = res[h]
            if t > 0:
                a = jnp.exp2(run[h][0] - m)
                o = run[h][1] * a + o
                sm = run[h][2] * a + sm
            run[h] = (m, o, sm)
            if t == j:
                gate = gate_ref[4 * g + h:4 * g + h + 1, :]
                if drained:
                    sm = jnp.where(never, drained.pop(), sm)
                l = jnp.sum(sm, axis=0, keepdims=True)
                r = mem[g, j // 2][:, 128 * (j % 2):128 * (j % 2) + 128]
                den = r[128 + h:129 + h] + 1e-6
                outs[h] = r[32 * h:32 * h + 32] * (gate / den) + o * ((1.0 - gate) / l)
        if t == j:
            ot = jnp.concatenate([outs[h] for h in range(4)], axis=0)
            ob = pltpu.bitcast(ot.T.astype(bf16), jnp.uint32)
            even = (lane // DH) % 2 == 0
            ob = jnp.concatenate([jnp.where(even, ob[32:64], ob[0:32]), jnp.where(even, ob[0:32], ob[32:64])], axis=0)
            o_ref[128 * j:128 * j + 128, 128 * g:128 * g + 128] = pltpu.bitcast(ob, bf16)
            drained.append(pltpu.bitcast(ob[56:64], f32))

    n_steps = len(steps)
    for n in range(n_steps + ATT_LAG):
        if n < n_steps:
            do_qk(n)
        for p in hooks.get(n, []):
            p()
        if n >= ATT_LAG:
            do_sm(n - ATT_LAG)
    for p in hooks.get(n_steps + ATT_LAG, []):
        p()


def _kernel(x_hbm, wq_hbm, wk_hbm, wv_hbm, wo_hbm, beta_hbm, w1_hbm, w2_hbm, w3_hbm, w4_hbm,
            out_hbm,
            xio, wqv_s, wk_v, wqvt, wo_v, w1_v, w2_v, w3_v, w4_v, beta_v,
            x_ref, y_ref, yc_ref, xn_ref, xc_ref, xa_ref,
            k_ref, pk_ref, qt_ref, pqt_ref, vt_ref, o_ref,
            mz_ref, mzmask_ref, mask_ref, gate_ref, zs_ref,
            sem_in, sem_x, sem_out):
    def cp(src, dst, i):
        return pltpu.make_async_copy(src, dst, sem_in.at[i])

    def x_cp(t):
        r0 = t * TB if isinstance(t, int) else pl.multiple_of(t * TB, TB)
        return pltpu.make_async_copy(x_hbm.at[pl.ds(r0, TB)], xio.at[pl.ds(r0, TB)], sem_x.at[t])

    def out_cp(t):
        r0 = t * TB if isinstance(t, int) else pl.multiple_of(t * TB, TB)
        return pltpu.make_async_copy(xio.at[pl.ds(r0, TB)], out_hbm.at[pl.ds(r0, TB)], sem_out.at[t])

    wqv_cp = [cp(w.at[:, pl.ds(HC * a, HC)], wqv_s.at[2 * a + i], 2 * a + i)
              for a in range(2) for i, w in enumerate((wq_hbm, wv_hbm))]
    wk_cp = [cp(wk_hbm.at[:, pl.ds(HC * a, HC)], wk_v.at[a], 4 + a) for a in range(2)]
    wo_cp = [cp(wo_hbm.at[pl.ds(HC * a, HC)], wo_v.at[a], 12 + a) for a in range(2)]
    beta_cp = cp(beta_hbm, beta_v, 6)
    w1_cp = cp(w1_hbm, w1_v, 8)
    w2_cp = cp(w2_hbm, w2_v, 9)
    w3_cp = cp(w3_hbm, w3_v, 10)
    w4_cp = cp(w4_hbm, w4_v, 11)

    for c in [beta_cp, x_cp(0), x_cp(1), wqv_cp[0]]:
        c.start()

    kk = lax.broadcasted_iota(jnp.int32, (64, 128), 0)
    qq = lax.broadcasted_iota(jnp.int32, (64, 128), 1)
    for i, q_pos in enumerate(((qq + 64) % 128, qq, qq % 64)):
        mask_ref[i] = jnp.where(kk <= q_pos, 0.0, NEG).astype(f32)
    rr = lax.broadcasted_iota(jnp.int32, (MZR, 128), 0)
    cc = lax.broadcasted_iota(jnp.int32, (MZR, 128), 1) // DH
    row_head = jnp.where(rr < 128, rr // DH, rr - 128)
    mzmask_ref[...] = jnp.where(row_head == cc, 1.0, 0.0).astype(f32)
    zs_ref[0] = jnp.int32(0)
    x_ref[0:YR, :] = jnp.zeros((YR, D), f32)
    x_ref[S:S + LNC, :] = jnp.zeros((LNC, D), f32)

    beta_cp.wait()
    eye = (lax.broadcasted_iota(jnp.int32, (H, H), 0) == lax.broadcasted_iota(jnp.int32, (H, H), 1))
    beta_rows = jnp.broadcast_to(beta_v[...].astype(f32), (H, H))
    beta_col = jnp.sum(jnp.where(eye, beta_rows, 0.0), axis=1, keepdims=True)
    gates = jnp.broadcast_to(jax.nn.sigmoid(beta_col), (H, 128))
    gate_ref[0] = gates[0:H // 2]
    gate_ref[1] = gates[H // 2:H]

    def loop(n, fn, name):
        def body(i, c):
            with jax.named_scope(name):
                fn(i)
            return c

        lax.fori_loop(0, n, body, 0)

    def never():
        return zs_ref[0] != 0

    def chunk(r0, i):
        return pl.ds(r0 + LNC * i if isinstance(r0, int) else pl.multiple_of(r0 + LNC * i, LNC), LNC)

    def norm_rows(r0, n, dsts):
        def load(i):
            return xio[chunk(r0, i), :].astype(f32)

        def post(i, y):
            for dst in dsts:
                dst[chunk(r0, i), :] = y.astype(bf16)
            return [y[r:r + 1, 0:128] for r in range(0, LNC, 8)]

        mean = _rowmean(xio[pl.ds(pl.multiple_of(r0, LNC), n), :].astype(f32))
        return functools.partial(_ln_chunks, mean, load, zs_ref[0], post)

    def mixer_norm(r0, n, dst, d0):
        def post(i, y):
            y_ref[chunk(r0, i), :] = y
            yn = _ln(y)
            dst[chunk(d0, i), :] = yn.astype(bf16)
            return [yn[r:r + 1, 0:128] for r in range(0, LNC, 8)]

        mean = _rowmean(x_ref[pl.ds(pl.multiple_of(r0, LNC), n), :])
        return functools.partial(_ln_chunks, mean, lambda i: x_ref[chunk(r0, i), :], zs_ref[0], post)

    def pt_body(layer, u):
        s = u // 2
        a = u % 2

        @pl.when(jnp.logical_and(layer == 0, u < 2))
        def _():
            ident = (lax.broadcasted_iota(jnp.int32, (128, 128), 0)
                     == lax.broadcasted_iota(jnp.int32, (128, 128), 1)).astype(bf16)
            src = [wqv_s.at[2 * u + i] for i in range(2)]
            for i in range(2):
                pltpu.make_async_copy(src[i], src[i], sem_in.at[2 * u + i]).wait()
            for n in range(2 * GH):
                g, i = divmod(n, 2)
                w = src[i][:, 128 * g:128 * g + 128]
                wqvt[u, g, 128 * i:128 * i + 128, :] = _dot_nt(ident, w).astype(bf16) if n in TR_MXU else w.T
            pltpu.make_async_copy(wk_v.at[u], wk_v.at[u], sem_in.at[4 + u]).wait()
            pltpu.make_async_copy(wo_v.at[u], wo_v.at[u], sem_in.at[12 + u]).wait()

            @pl.when(u == 0)
            def _():
                for c in [wqv_cp[2], wqv_cp[3], wk_cp[1], wo_cp[1], x_cp(3)]:
                    c.start()

            @pl.when(u == 1)
            def _():
                for c in [x_cp(t) for t in range(4, S // TB)] + [w1_cp]:
                    c.start()

        @pl.when(jnp.logical_and(layer == 0, u < S // TB - 2))
        def _():
            x_cp(u + 2).wait()

            @pl.when(u == 2)
            def _():
                w2_cp.start()
                w3_cp.start()

            @pl.when(u == 4)
            def _():
                w4_cp.start()

        r0 = pl.multiple_of(s * L, L)
        g0 = GH * a
        mem, run, ties = {}, {}, {}

        y0 = jnp.clip((u - 2) * YR, 0, TB + LNC - YR)
        norms = {"x": norm_rows(((s + 1) % NSEG) * L + a * TB, TB, [xn_ref]),
                 "y": mixer_norm(y0, YR, yc_ref, y0 + LNC)}

        def norm(kind, sel, due):
            after = jnp.concatenate([run[0][2][:, 0:1]] * (LNC // 8), axis=0) if run else None
            for i, v in enumerate(norms[kind](after, sel)):
                ties.setdefault(due + i, []).extend(v)

        def qv_proj(g, c):
            gs, cs = slice(128 * g, 128 * g + 128), slice(128 * c, 128 * c + 128)
            r = _dot_nt(wqvt[a, g], xc_ref[cs, :])
            q = jnp.concatenate([r[32 * h:32 * h + 32] if h % 2 else pltpu.roll(r[32 * h:32 * h + 32], 64, 1)
                                 for h in range(4)], axis=0)
            qt_ref[gs, cs] = (q * QSCALE).astype(bf16)
            pqt_ref[gs, cs] = _phi(q).astype(bf16)
            vt_ref[gs, cs] = r[128:256].astype(bf16)

        def k_proj(g, c):
            gs, rs = slice(128 * g, 128 * g + 128), slice(256 * c, 256 * c + 256)
            kf = _dot(xc_ref[rs, :], wk_v[a, :, gs])
            k_ref[rs, gs] = kf.astype(bf16)
            pk_ref[rs, gs] = _phi(kf).astype(bf16)

        def retrieve(g, c):
            mzb = mz_ref[g0 + g].astype(bf16)
            mem[g, c] = jnp.concatenate([
                jnp.concatenate([_dot(mzb[rs], pqt_ref[128 * g:128 * g + 128, 128 * j:128 * j + 128])
                                 for rs in (slice(0, r), slice(r, MZR))], axis=0)
                for j, r in ((2 * c, 64 + 16 * c), (2 * c + 1, 64 + 16 * c))], axis=1)

        def mem_update(g):
            ones = jnp.ones((MZR - 128, L), bf16)
            lhs = jnp.concatenate([vt_ref[128 * g:128 * g + 128, :], ones], axis=0)
            upd = _dot(lhs, pk_ref[:, 128 * g:128 * g + 128])
            mz_ref[g0 + g] = jnp.where(s == NSEG - 1, 0.0, mz_ref[g0 + g] + upd * mzmask_ref[...])

        def out_proj(part, j):
            rows = pl.ds(pl.multiple_of(r0 + 128 * j, 128), 128)
            rs, ks = slice(128 * j, 128 * j + 128), slice(256 * part, 256 * part + 256)
            upd = _dot(o_ref[rs, ks], wo_v[a, ks, :])
            if part == 0:
                xa_ref[rs, :] = upd
            else:
                base = jnp.where(a == 0, xio[rows, :].astype(f32), x_ref[rows, :])
                x_ref[rows, :] = base + xa_ref[rs, :] + upd
                nxt = ((u + 1) // 2) % NSEG
                xc_ref[rs, :] = _paced(xn_ref[pl.ds(pl.multiple_of(nxt * L + 128 * j, 128), 128), :], upd, never())

        work = {"qv": qv_proj, "k": k_proj, "ret": retrieve, "mem": mem_update, "wo": out_proj,
                "ln": norm}
        hooks = {}
        for n, kind, *args in SCHEDULE:
            hooks.setdefault(n, []).append(functools.partial(work[kind], *args))
        for p in hooks.pop(-1):
            p()
        _attention(k_ref, qt_ref, vt_ref, mem, run, gate_ref.at[a], mask_ref, o_ref, hooks, ties,
                   never())

    def mix_body(layer, t):
        r0 = pl.multiple_of(t * TB, TB)
        half = TB // 2
        cols = range(0, D, 128)

        def tiles(x):
            return [x[r:r + 16] for r in range(0, half, 16)]

        def shifted(a):
            n = half // 2 + LNC
            win = pltpu.bitcast(yc_ref[half * a:half * a + 2 * n, :], jnp.uint32)
            mid = slice(LNC // 2, LNC // 2 + half // 2)
            prv, cur, nxt = pltpu.roll(win, 1, 0)[mid], win[mid], pltpu.roll(win, n - 1, 0)[mid]
            return [pltpu.bitcast(v, bf16)
                    for v in ((prv >> 16) | (cur << 16), (cur >> 16) | (nxt << 16), prv, nxt)]

        hs = []
        for a in range(2):
            lhs = shifted(a)
            hq = {c: _gelu(_dot(lhs[4 * c // D], w1_v[:, c:c + 128])).astype(bf16) for c in W1_ORDER}
            hs.append(jnp.concatenate([hq[c] for c in cols], axis=1))
        yc_ref[0:2 * LNC, :] = yc_ref[TB:TB + 2 * LNC, :]

        def norm(a, upd, gates):
            ra = pl.multiple_of(r0 + half * a, half)
            x1 = y_ref[pl.ds(ra, half), :] + jnp.concatenate(upd, axis=1)
            xa_ref[half * a:half * a + half, :] = x1
            mean = _rowmean(x1)
            out = []
            for i in range(half // LNC):
                gate = gates[i - LN_LEAD][0:LNC, 0:1] if i >= LN_LEAD else None
                out += _ln_chunks(mean, lambda i: xa_ref[pl.ds(half * a + LNC * i, LNC), :], zs_ref[0],
                                  lambda i, y: y.astype(bf16), gate, (i,))
            return jnp.concatenate(out, axis=0)

        def up(lhs, c):
            return _gelu(_dot(lhs, w3_v[:, FC * c:FC * c + FC]))

        upd0 = [_dot(_after(hs[0], tiles(hs[1][:, c - 128:c]), never()) if c else hs[0], w2_v[:, c:c + 128])
                for c in cols]
        upd1 = [_dot(hs[1], w2_v[:, c:c + 128]) for c in cols]
        x1n = [norm(0, upd0, upd1)]
        pre = [_dot(x1n[0], w3_v[:, c:c + 128]) for c in range(0, 2 * FC, 128)]
        x1n.append(norm(1, upd1, pre))
        pre = _gelu(jnp.concatenate(pre, axis=1))
        nch = F // FC
        x1n_full = jnp.concatenate(x1n, axis=0)
        hid = {c: jnp.concatenate([pre[:, FC * c:FC * c + FC], up(x1n[1], c)], axis=0).astype(bf16)
               for c in range(2)}
        acc = x_ref[pl.ds(r0, TB), :] + xa_ref[0:TB, :]
        xr = (nch - 2) * LNC
        next_norm = norm_rows(jnp.clip((t - 1) * xr, 0, L - xr), xr, [xn_ref, xc_ref])
        next_mix = mixer_norm(jnp.minimum(r0 + TB, S - TB) + LNC, TB, yc_ref, 2 * LNC)
        done = []
        for c in range(nch):
            down = _dot(hid.pop(c), w4_v[FC * c:FC * c + FC, :])
            acc = acc + down
            sel = [i for i, n in enumerate(MIX_LN) if n == c]
            if c + 2 < nch:
                act = up(x1n_full, c + 2)
                hid[c + 2] = act.astype(bf16)
                done += next_norm(act[0:LNC, 0:1], [c])
            else:
                act = down
            if sel:
                done += next_mix(act[0:LNC, 0:1], sel)
            due = min(c + 2, nch - 1)
            if c != nch - 3 and due in hid:
                hid[due] = _after(hid[due], sum(done, []), never())
                done = []
        xio[pl.ds(r0, TB), :] = acc.astype(bf16)

        @pl.when(layer == 1)
        def _():
            out_cp(t).start()

    def norm0(i):
        x_cp(i).wait()

        @pl.when(i == 0)
        def _():
            wqv_cp[1].start()

        @pl.when(i == 1)
        def _():
            wk_cp[0].start()
            wo_cp[0].start()
            x_cp(2).start()

        rows = pl.ds(pl.multiple_of(i * TB, TB), TB)
        xn = _ln(xio[rows, :].astype(f32)).astype(bf16)
        xn_ref[rows, :] = xn
        xc_ref[rows, :] = xn

    mz_ref[...] = jnp.zeros(mz_ref.shape, f32)
    loop(L // TB, norm0, "norm0")

    def layer_body(layer):
        loop(2 * NSEG, lambda u: pt_body(layer, u), "pt")

        @pl.when(layer == 0)
        def _():
            w1_cp.wait()
            w2_cp.wait()
            w3_cp.wait()
            w4_cp.wait()

        yc_ref[0:LNC, :] = jnp.zeros((LNC, D), bf16)

        loop(S // TB, lambda t: mix_body(layer, t), "mix")

    loop(2, layer_body, "layer")
    for t in range(S // TB):
        out_cp(t).wait()


@jax.jit
def pallas_interleave_layers__memory_aug_infini_attn__mixer_s_mlp__prompt_kernel(
    A_x: jax.Array,
    A_wq: jax.Array,
    A_wk: jax.Array,
    A_wv: jax.Array,
    A_wo: jax.Array,
    A_beta: jax.Array,
    B_x: jax.Array,
    B_w1: jax.Array,
    B_w2: jax.Array,
    B_w3: jax.Array,
    B_w4: jax.Array,
):
    del B_x
    x = A_x.reshape(S, D)
    beta = A_beta.reshape(1, H)
    any_spec = pl.BlockSpec(memory_space=pl.ANY)
    scratch = [
        pltpu.VMEM((S, D), bf16),
        pltpu.VMEM((4, D, HC), bf16),
        pltpu.VMEM((2, D, HC), bf16),
        pltpu.VMEM((2, GH, 256, D), bf16),
        pltpu.VMEM((2, HC, D), bf16),
        pltpu.VMEM((D, D), bf16),
        pltpu.VMEM((D, D), bf16),
        pltpu.VMEM((D, F), bf16),
        pltpu.VMEM((F, D), bf16),
        pltpu.VMEM((1, H), bf16),
        pltpu.VMEM((S + LNC, D), f32),
        pltpu.VMEM((S + LNC, D), f32),
        pltpu.VMEM((TB + 2 * LNC, D), bf16),
        pltpu.VMEM((S, D), bf16),
        pltpu.VMEM((L, D), bf16),
        pltpu.VMEM((L, D), f32),
        pltpu.VMEM((L, HC), bf16),
        pltpu.VMEM((L, HC), bf16),
        pltpu.VMEM((HC, L), bf16),
        pltpu.VMEM((HC, L), bf16),
        pltpu.VMEM((HC, L), bf16),
        pltpu.VMEM((L, HC), bf16),
        pltpu.VMEM((NG, MZR, 128), f32),
        pltpu.VMEM((MZR, 128), f32),
        pltpu.VMEM((3, 64, 128), f32),
        pltpu.VMEM((2, H // 2, 128), f32),
        pltpu.SMEM((1,), jnp.int32),
        pltpu.SemaphoreType.DMA((14,)),
        pltpu.SemaphoreType.DMA((S // TB,)),
        pltpu.SemaphoreType.DMA((S // TB,)),
    ]
    out = pl.pallas_call(
        _kernel,
        out_shape=jax.ShapeDtypeStruct((S, D), bf16),
        in_specs=[any_spec] * 10,
        out_specs=any_spec,
        scratch_shapes=scratch,
        compiler_params=pltpu.CompilerParams(vmem_limit_bytes=112 * 1024 * 1024),
    )(x, A_wq, A_wk, A_wv, A_wo, beta, B_w1, B_w2, B_w3, B_w4)
    return out.reshape(1, S, D)
```

```python
import functools
import math

import jax
import jax.numpy as jnp
from jax import lax
import jax.experimental.pallas as pl
import jax.experimental.pallas.tpu as pltpu

f32 = jnp.float32
bf16 = jnp.bfloat16

S = 2048
D = 1024
F = 3584
H = 32
DH = 32
L = 512
NSEG = S // L
NG = D // 128
HC = D // 2
GH = HC // 128
TB = 256
FC = 512
MZR = 144
EPS = 1e-5
NEG = -1e30
QSCALE = (DH ** -0.5) * math.log2(math.e)
GELU_C0 = math.sqrt(2.0 / math.pi)
GELU_C1 = GELU_C0 * 0.044715
ATT_LAG = 2
LN_LEAD = 2
MIX_LN = (0, 0, 1, 1, 2, 2, 3, 3, 4, 4, 5, 5, 5, 6, 6, 6)
LNC = 16
DIAG_ORDER = ((0, 2, 1, 3), (2, 0, 3, 1))
QROLL = (64, 0, 32, 96)
TR_MXU = (0, 3, 6)
W1_ORDER = (512, 640, 768, 896, 0, 128, 256, 384)
YR = 48
SCHEDULE = (
    (-1, "ln", "y", (0, 1, 2), 0), (-1, "k", 0, 0), (-1, "qv", 0, 0), (-1, "qv", 0, 1), (0, "qv", 0, 2),
    (0, "k", 0, 1), (1, "ret", 0, 0), (4, "qv", 0, 3), (4, "k", 1, 0), (5, "ret", 0, 1), (7, "qv", 1, 0),
    (9, "qv", 1, 1), (11, "ret", 1, 0), (11, "qv", 1, 2), (11, "k", 1, 1), (12, "ln", "x", (0,), 13),
    (13, "ln", "x", (1,), 14), (14, "qv", 1, 3), (14, "k", 2, 0), (14, "ln", "x", (2,), 15),
    (15, "ln", "x", (3,), 16), (16, "ret", 1, 1), (16, "wo", 0, 0), (19, "qv", 2, 0), (19, "qv", 2, 1),
    (20, "ret", 2, 0), (21, "qv", 2, 3), (21, "ln", "x", (4,), 22), (21, "qv", 2, 2),
    (21, "ln", "x", (6,), 22), (22, "k", 2, 1), (22, "ln", "x", (5,), 23), (23, "k", 3, 0),
    (25, "ln", "x", (7,), 26), (25, "ln", "x", (9,), 26), (25, "ln", "x", (8,), 26), (26, "wo", 0, 1),
    (27, "ret", 2, 1), (27, "qv", 3, 0), (27, "ln", "x", (10,), 28), (28, "ln", "x", (11,), 29),
    (30, "qv", 3, 1), (30, "qv", 3, 2), (30, "ret", 3, 0), (30, "ln", "x", (12,), 31), (31, "qv", 3, 3),
    (31, "ln", "x", (13,), 32), (33, "k", 3, 1), (33, "mem", 0), (33, "ln", "x", (15,), 34), (35, "wo", 0, 2),
    (35, "wo", 0, 3), (36, "ln", "x", (14,), 37), (36, "wo", 1, 0), (36, "mem", 1), (37, "ret", 3, 1),
    (40, "mem", 3), (40, "wo", 1, 1), (41, "mem", 2), (42, "wo", 1, 2), (42, "wo", 1, 3),
)


def _dot(a, b):
    return jnp.dot(a, b, preferred_element_type=f32)


def _dot_nt(a, b):
    return lax.dot_general(a, b, (((1,), (1,)), ((), ())), preferred_element_type=f32)


def _ln(x):
    m = jnp.mean(x, axis=-1, keepdims=True)
    xc = x - m
    v = jnp.mean(xc * xc, axis=-1, keepdims=True)
    return xc * lax.rsqrt(v + EPS)


def _ln_chunks(mean, load, zero, post, prev=None, sel=None):
    outs = []
    for i in sel or range(mean.shape[0] // LNC):
        m = mean[LNC * i:LNC * i + LNC]
        if prev is not None:
            m = pltpu.bitcast(pltpu.bitcast(m, jnp.int32) | (pltpu.bitcast(prev, jnp.int32) & zero), f32)
        xc = load(i) - m
        prev = lax.rsqrt(jnp.mean(xc * xc, axis=-1, keepdims=True) + EPS)
        outs.append(post(i, xc * prev))
    return outs


def _rowmean(x):
    return jnp.mean(x, axis=-1, keepdims=True)


def _gelu(x):
    t = jnp.tanh(x * (GELU_C0 + GELU_C1 * (x * x)))
    hx = 0.5 * x
    return hx + hx * t


def _phi(t):
    return jnp.where(t > 0, t + 1.0, jnp.exp(t))


def _fold(x, op):
    parts = [x[8 * i:8 * i + 8] for i in range(x.shape[0] // 8)]
    while len(parts) > 1:
        parts = [op(parts[i], parts[i + 1]) for i in range(0, len(parts), 2)]
    return parts[0]


def _after(x, deps, never):
    d = functools.reduce(jnp.bitwise_or, [pltpu.bitcast(v, jnp.uint32) for v in deps])
    bits = pltpu.bitcast(x, jnp.uint32)
    top = jnp.concatenate([jnp.where(never, d, bits[0:8, 0:128]), bits[0:8, 128:]], axis=1)
    return pltpu.bitcast(jnp.concatenate([top, bits[8:]], axis=0), x.dtype)


def _paced(x, pace, never):
    bits = pltpu.bitcast(x, jnp.uint32)
    return pltpu.bitcast(jnp.where(never, pltpu.bitcast(pace[0:bits.shape[0]], jnp.uint32), bits), x.dtype)


def _attention(k_ref, qt_ref, vt_ref, mem, run, gate_ref, mask_ref, o_ref, hooks, ties, never):
    steps = [(g, j, t) for g in range(GH) for j in range(4) for t in range(j + 1)]
    scores, outs = {}, {}
    drained = []

    lane = lax.broadcasted_iota(jnp.int32, (1, 128), 1)
    late = [[(lane + 128 - r) % 128 >= b for r in QROLL] for b in (64, 96)]

    def keep(x, h, i):
        bits = pltpu.bitcast(x, jnp.uint32)
        return pltpu.bitcast(jnp.where(late[i][h], bits, jnp.uint32(0)), bf16)

    def pad(x, r):
        parts = [jnp.zeros((r, 128), bf16), x, jnp.zeros((128 - r - x.shape[0], 128), bf16)]
        return jnp.concatenate([v for v in parts if v.shape[0]], axis=0)

    def do_qk(n):
        g, j, t = steps[n]
        gs = slice(128 * g, 128 * g + 128)
        q = [qt_ref[128 * g + 32 * h:128 * g + 32 * h + 32, 128 * j:128 * j + 128] for h in range(4)]
        w = jnp.concatenate([pad(q[h], 32 * h) for h in range(4)], axis=1)
        if t < j:
            scores[n] = (_dot(k_ref[128 * t:128 * t + 128, gs], w), None)
            return
        w2 = [pad(jnp.concatenate([keep(q[h], h, 0), keep(q[h + 1], h + 1, 0)], axis=0), 32 * h) for h in (0, 2)]
        w3 = jnp.concatenate([keep(q[h], h, 1) for h in range(4)], axis=0)
        s1 = _dot(k_ref[128 * t:128 * t + 64, gs], w)
        parts = [(64, 32, w2[0]), (64, 32, w2[1]), (96, 16, w3), (112, 16, w3)]
        order = DIAG_ORDER[j % len(DIAG_ORDER)]
        d = {i: _dot(k_ref[128 * t + parts[i][0]:128 * t + parts[i][0] + parts[i][1], gs], parts[i][2]) for i in order}
        s2 = [d[0], d[1], jnp.concatenate([d[2], d[3]], axis=0)]
        scores[n] = (s1, jnp.concatenate(s2, axis=1))

    def do_sm(n):
        g, j, t = steps[n]
        st, st2 = scores.pop(n)
        cur = []
        if t == j:
            st2 = [st2[:, 128 * i:128 * i + 128] + mask_ref[4 + i, 0:32] for i in range(3)]
            mx2 = [_fold(v, jnp.maximum) for v in st2]
        for h in range(4):
            s = st[:, 128 * h:128 * h + 128]
            if t == j:
                s = s + mask_ref[h]
            mx = _fold(s, jnp.maximum)
            if t == j:
                mx = jnp.where(late[0][h], jnp.maximum(mx, mx2[h // 2]), mx)
                mx = jnp.where(late[1][h], jnp.maximum(mx, mx2[2]), mx)
            m = jnp.max(mx, axis=0, keepdims=True)
            if t > 0:
                m = jnp.maximum(m, run[h][0])
            if h == 0 and n in ties:
                m = jnp.where(never, functools.reduce(jnp.add, ties[n]), m)
            cur.append((s, m))
        res = []
        if t == j:
            m2 = [jnp.where(late[0][h], cur[h][1], cur[h + 1][1]) for h in (0, 2)]
            m2.append(jnp.where(jnp.logical_or(late[1][0], late[1][1]), m2[0], m2[1]))
            p2 = [jnp.exp2(v - m) for v, m in zip(st2, m2)]
            sm2, pb2 = [_fold(v, jnp.add) for v in p2], [v.astype(bf16) for v in p2]
        for h in range(4):
            s, m = cur[h]
            r0 = 128 * g + 32 * h
            p = jnp.exp2(s - m)
            sm = _fold(p, jnp.add)
            pb = p.astype(bf16)
            if t == j:
                sm = jnp.where(late[0][h], sm + sm2[h // 2], sm)
                sm = jnp.where(late[1][h], sm + sm2[2], sm)
                pb = jnp.concatenate([pb, keep(pb2[h // 2], h, 0), keep(pb2[2], h, 1)], axis=0)
            o = _dot(vt_ref[r0:r0 + 32, 128 * t:128 * t + 128], pb)
            res.append((m, o, sm))
        for h in range(4):
            m, o, sm = res[h]
            if t > 0:
                a = jnp.exp2(run[h][0] - m)
                o = run[h][1] * a + o
                sm = run[h][2] * a + sm
            run[h] = (m, o, sm)
            if t == j:
                gate = gate_ref[4 * g + h:4 * g + h + 1, :]
                if drained:
                    sm = jnp.where(never, drained.pop(), sm)
                l = jnp.sum(sm, axis=0, keepdims=True)
                r = mem[g, j // 2][:, 128 * (j % 2):128 * (j % 2) + 128]
                den = r[128 + h:129 + h] + 1e-6
                outs[h] = r[32 * h:32 * h + 32] * (gate / den) + o * ((1.0 - gate) / l)
        if t == j:
            ot = jnp.concatenate([outs[h] for h in range(4)], axis=0)
            ob = pltpu.bitcast(ot.T.astype(bf16), jnp.uint32)
            far = (lane + 96) % 128 >= 64
            ob = jnp.concatenate([jnp.where(far, ob[32:64], ob[0:32]), jnp.where(far, ob[0:32], ob[32:64])], axis=0)
            ob = jnp.where(lane >= 64, jnp.concatenate([ob[16:64], ob[0:16]], axis=0), ob)
            o_ref[128 * j:128 * j + 128, 128 * g:128 * g + 128] = pltpu.bitcast(ob, bf16)
            drained.append(pltpu.bitcast(ob[56:64], f32))

    n_steps = len(steps)
    for n in range(n_steps + ATT_LAG):
        if n < n_steps:
            do_qk(n)
        for p in hooks.get(n, []):
            p()
        if n >= ATT_LAG:
            do_sm(n - ATT_LAG)
    for p in hooks.get(n_steps + ATT_LAG, []):
        p()


def _kernel(x_hbm, wq_hbm, wk_hbm, wv_hbm, wo_hbm, beta_hbm, w1_hbm, w2_hbm, w3_hbm, w4_hbm,
            out_hbm,
            xio, wqv_s, wk_v, wqvt, wo_v, w1_v, w2_v, w3_v, w4_v, beta_v,
            x_ref, y_ref, yc_ref, xn_ref, xc_ref, xa_ref,
            k_ref, pk_ref, qt_ref, pqt_ref, vt_ref, o_ref,
            mz_ref, mzmask_ref, mask_ref, gate_ref, zs_ref,
            sem_in, sem_x, sem_out):
    def cp(src, dst, i):
        return pltpu.make_async_copy(src, dst, sem_in.at[i])

    def x_cp(t):
        r0 = t * TB if isinstance(t, int) else pl.multiple_of(t * TB, TB)
        return pltpu.make_async_copy(x_hbm.at[pl.ds(r0, TB)], xio.at[pl.ds(r0, TB)], sem_x.at[t])

    def out_cp(t):
        r0 = t * TB if isinstance(t, int) else pl.multiple_of(t * TB, TB)
        return pltpu.make_async_copy(xio.at[pl.ds(r0, TB)], out_hbm.at[pl.ds(r0, TB)], sem_out.at[t])

    wqv_cp = [cp(w.at[:, pl.ds(HC * a, HC)], wqv_s.at[2 * a + i], 2 * a + i)
              for a in range(2) for i, w in enumerate((wq_hbm, wv_hbm))]
    wk_cp = [cp(wk_hbm.at[:, pl.ds(HC * a, HC)], wk_v.at[a], 4 + a) for a in range(2)]
    wo_cp = [cp(wo_hbm.at[pl.ds(HC * a, HC)], wo_v.at[a], 12 + a) for a in range(2)]
    beta_cp = cp(beta_hbm, beta_v, 6)
    w1_cp = cp(w1_hbm, w1_v, 8)
    w2_cp = cp(w2_hbm, w2_v, 9)
    w3_cp = cp(w3_hbm, w3_v, 10)
    w4_cp = cp(w4_hbm, w4_v, 11)

    for c in [beta_cp, x_cp(0), x_cp(1), wqv_cp[0]]:
        c.start()

    kk = lax.broadcasted_iota(jnp.int32, (64, 128), 0)
    qq = lax.broadcasted_iota(jnp.int32, (64, 128), 1)
    for i, q_pos in enumerate([(qq + 128 - r) % 128 for r in QROLL] + [qq % 64, (qq + 32) % 64, qq % 32]):
        mask_ref[i] = jnp.where(kk <= q_pos, 0.0, NEG).astype(f32)
    rr = lax.broadcasted_iota(jnp.int32, (MZR, 128), 0)
    cc = lax.broadcasted_iota(jnp.int32, (MZR, 128), 1) // DH
    row_head = jnp.where(rr < 128, rr // DH, rr - 128)
    mzmask_ref[...] = jnp.where(row_head == cc, 1.0, 0.0).astype(f32)
    zs_ref[0] = jnp.int32(0)
    x_ref[0:YR, :] = jnp.zeros((YR, D), f32)
    x_ref[S:S + LNC, :] = jnp.zeros((LNC, D), f32)

    beta_cp.wait()
    eye = (lax.broadcasted_iota(jnp.int32, (H, H), 0) == lax.broadcasted_iota(jnp.int32, (H, H), 1))
    beta_rows = jnp.broadcast_to(beta_v[...].astype(f32), (H, H))
    beta_col = jnp.sum(jnp.where(eye, beta_rows, 0.0), axis=1, keepdims=True)
    gates = jnp.broadcast_to(jax.nn.sigmoid(beta_col), (H, 128))
    gate_ref[0] = gates[0:H // 2]
    gate_ref[1] = gates[H // 2:H]

    def loop(n, fn, name):
        def body(i, c):
            with jax.named_scope(name):
                fn(i)
            return c

        lax.fori_loop(0, n, body, 0)

    def never():
        return zs_ref[0] != 0

    def chunk(r0, i):
        return pl.ds(r0 + LNC * i if isinstance(r0, int) else pl.multiple_of(r0 + LNC * i, LNC), LNC)

    def norm_rows(r0, n, dsts):
        def load(i):
            return xio[chunk(r0, i), :].astype(f32)

        def post(i, y):
            for dst in dsts:
                dst[chunk(r0, i), :] = y.astype(bf16)
            return [y[r:r + 1, 0:128] for r in range(0, LNC, 8)]

        mean = _rowmean(xio[pl.ds(pl.multiple_of(r0, LNC), n), :].astype(f32))
        return functools.partial(_ln_chunks, mean, load, zs_ref[0], post)

    def mixer_norm(r0, n, dst, d0):
        def post(i, y):
            y_ref[chunk(r0, i), :] = y
            yn = _ln(y)
            dst[chunk(d0, i), :] = yn.astype(bf16)
            return [yn[r:r + 1, 0:128] for r in range(0, LNC, 8)]

        mean = _rowmean(x_ref[pl.ds(pl.multiple_of(r0, LNC), n), :])
        return functools.partial(_ln_chunks, mean, lambda i: x_ref[chunk(r0, i), :], zs_ref[0], post)

    def pt_body(layer, u):
        s = u // 2
        a = u % 2

        @pl.when(jnp.logical_and(layer == 0, u < 2))
        def _():
            ident = (lax.broadcasted_iota(jnp.int32, (128, 128), 0)
                     == lax.broadcasted_iota(jnp.int32, (128, 128), 1)).astype(bf16)
            src = [wqv_s.at[2 * u + i] for i in range(2)]
            for i in range(2):
                pltpu.make_async_copy(src[i], src[i], sem_in.at[2 * u + i]).wait()
            for n in range(2 * GH):
                g, i = divmod(n, 2)
                w = src[i][:, 128 * g:128 * g + 128]
                wqvt[u, g, 128 * i:128 * i + 128, :] = _dot_nt(ident, w).astype(bf16) if n in TR_MXU else w.T
            pltpu.make_async_copy(wk_v.at[u], wk_v.at[u], sem_in.at[4 + u]).wait()
            pltpu.make_async_copy(wo_v.at[u], wo_v.at[u], sem_in.at[12 + u]).wait()

            @pl.when(u == 0)
            def _():
                for c in [wqv_cp[2], wqv_cp[3], wk_cp[1], wo_cp[1], x_cp(3)]:
                    c.start()

            @pl.when(u == 1)
            def _():
                for c in [x_cp(t) for t in range(4, S // TB)] + [w1_cp]:
                    c.start()

        @pl.when(jnp.logical_and(layer == 0, u < S // TB - 2))
        def _():
            x_cp(u + 2).wait()

            @pl.when(u == 2)
            def _():
                w2_cp.start()
                w3_cp.start()

            @pl.when(u == 4)
            def _():
                w4_cp.start()

        r0 = pl.multiple_of(s * L, L)
        g0 = GH * a
        mem, run, ties = {}, {}, {}

        y0 = jnp.clip((u - 2) * YR, 0, TB + LNC - YR)
        norms = {"x": norm_rows(((s + 1) % NSEG) * L + a * TB, TB, [xn_ref]),
                 "y": mixer_norm(y0, YR, yc_ref, y0 + LNC)}

        def norm(kind, sel, due):
            after = jnp.concatenate([run[0][2][:, 0:1]] * (LNC // 8), axis=0) if run else None
            for i, v in enumerate(norms[kind](after, sel)):
                ties.setdefault(due + i, []).extend(v)

        def qv_proj(g, c):
            gs, cs = slice(128 * g, 128 * g + 128), slice(128 * c, 128 * c + 128)
            r = _dot_nt(wqvt[a, g], xc_ref[cs, :])
            q = jnp.concatenate([pltpu.roll(r[32 * h:32 * h + 32], QROLL[h], 1) if QROLL[h] else r[32 * h:32 * h + 32]
                                 for h in range(4)], axis=0)
            qt_ref[gs, cs] = (q * QSCALE).astype(bf16)
            pqt_ref[gs, cs] = _phi(q).astype(bf16)
            vt_ref[gs, cs] = r[128:256].astype(bf16)

        def k_proj(g, c):
            gs, rs = slice(128 * g, 128 * g + 128), slice(256 * c, 256 * c + 256)
            kf = _dot(xc_ref[rs, :], wk_v[a, :, gs])
            k_ref[rs, gs] = kf.astype(bf16)
            pk_ref[rs, gs] = _phi(kf).astype(bf16)

        def retrieve(g, c):
            mzb = mz_ref[g0 + g].astype(bf16)
            mem[g, c] = jnp.concatenate([
                jnp.concatenate([_dot(mzb[rs], pqt_ref[128 * g:128 * g + 128, 128 * j:128 * j + 128])
                                 for rs in (slice(0, r), slice(r, MZR))], axis=0)
                for j, r in ((2 * c, 64 + 16 * c), (2 * c + 1, 64 + 16 * c))], axis=1)

        def mem_update(g):
            ones = jnp.ones((MZR - 128, L), bf16)
            lhs = jnp.concatenate([vt_ref[128 * g:128 * g + 128, :], ones], axis=0)
            upd = _dot(lhs, pk_ref[:, 128 * g:128 * g + 128])
            mz_ref[g0 + g] = jnp.where(s == NSEG - 1, 0.0, mz_ref[g0 + g] + upd * mzmask_ref[...])

        def out_proj(part, j):
            rows = pl.ds(pl.multiple_of(r0 + 128 * j, 128), 128)
            rs, ks = slice(128 * j, 128 * j + 128), slice(256 * part, 256 * part + 256)
            upd = _dot(o_ref[rs, ks], wo_v[a, ks, :])
            if part == 0:
                xa_ref[rs, :] = upd
            else:
                base = jnp.where(a == 0, xio[rows, :].astype(f32), x_ref[rows, :])
                x_ref[rows, :] = base + xa_ref[rs, :] + upd
                nxt = ((u + 1) // 2) % NSEG
                xc_ref[rs, :] = _paced(xn_ref[pl.ds(pl.multiple_of(nxt * L + 128 * j, 128), 128), :], upd, never())

        work = {"qv": qv_proj, "k": k_proj, "ret": retrieve, "mem": mem_update, "wo": out_proj,
                "ln": norm}
        hooks = {}
        for n, kind, *args in SCHEDULE:
            hooks.setdefault(n, []).append(functools.partial(work[kind], *args))
        for p in hooks.pop(-1):
            p()
        _attention(k_ref, qt_ref, vt_ref, mem, run, gate_ref.at[a], mask_ref, o_ref, hooks, ties,
                   never())

    def mix_body(layer, t):
        r0 = pl.multiple_of(t * TB, TB)
        half = TB // 2
        cols = range(0, D, 128)

        def tiles(x):
            return [x[r:r + 16] for r in range(0, half, 16)]

        def shifted(a):
            n = half // 2 + LNC
            win = pltpu.bitcast(yc_ref[half * a:half * a + 2 * n, :], jnp.uint32)
            mid = slice(LNC // 2, LNC // 2 + half // 2)
            prv, cur, nxt = pltpu.roll(win, 1, 0)[mid], win[mid], pltpu.roll(win, n - 1, 0)[mid]
            return [pltpu.bitcast(v, bf16)
                    for v in ((prv >> 16) | (cur << 16), (cur >> 16) | (nxt << 16), prv, nxt)]

        hs = []
        for a in range(2):
            lhs = shifted(a)
            hq = {c: _gelu(_dot(lhs[4 * c // D], w1_v[:, c:c + 128])).astype(bf16) for c in W1_ORDER}
            hs.append(jnp.concatenate([hq[c] for c in cols], axis=1))
        yc_ref[0:2 * LNC, :] = yc_ref[TB:TB + 2 * LNC, :]

        def norm(a, upd, gates):
            ra = pl.multiple_of(r0 + half * a, half)
            x1 = y_ref[pl.ds(ra, half), :] + jnp.concatenate(upd, axis=1)
            xa_ref[half * a:half * a + half, :] = x1
            mean = _rowmean(x1)
            out = []
            for i in range(half // LNC):
                gate = gates[i - LN_LEAD][0:LNC, 0:1] if i >= LN_LEAD else None
                out += _ln_chunks(mean, lambda i: xa_ref[pl.ds(half * a + LNC * i, LNC), :], zs_ref[0],
                                  lambda i, y: y.astype(bf16), gate, (i,))
            return jnp.concatenate(out, axis=0)

        def up(lhs, c):
            return _gelu(_dot(lhs, w3_v[:, FC * c:FC * c + FC]))

        upd0 = [_dot(_after(hs[0], tiles(hs[1][:, c - 128:c]), never()) if c else hs[0], w2_v[:, c:c + 128])
                for c in cols]
        upd1 = [_dot(hs[1], w2_v[:, c:c + 128]) for c in cols]
        x1n = [norm(0, upd0, upd1)]
        pre = [_dot(x1n[0], w3_v[:, c:c + 128]) for c in range(0, 2 * FC, 128)]
        x1n.append(norm(1, upd1, pre))
        pre = _gelu(jnp.concatenate(pre, axis=1))
        nch = F // FC
        x1n_full = jnp.concatenate(x1n, axis=0)
        hid = {c: jnp.concatenate([pre[:, FC * c:FC * c + FC], up(x1n[1], c)], axis=0).astype(bf16)
               for c in range(2)}
        acc = x_ref[pl.ds(r0, TB), :] + xa_ref[0:TB, :]
        xr = (nch - 2) * LNC
        next_norm = norm_rows(jnp.clip((t - 1) * xr, 0, L - xr), xr, [xn_ref, xc_ref])
        next_mix = mixer_norm(jnp.minimum(r0 + TB, S - TB) + LNC, TB, yc_ref, 2 * LNC)
        done = []
        for c in range(nch):
            down = _dot(hid.pop(c), w4_v[FC * c:FC * c + FC, :])
            acc = acc + down
            sel = [i for i, n in enumerate(MIX_LN) if n == c]
            if c + 2 < nch:
                act = up(x1n_full, c + 2)
                hid[c + 2] = act.astype(bf16)
                done += next_norm(act[0:LNC, 0:1], [c])
            else:
                act = down
            if sel:
                done += next_mix(act[0:LNC, 0:1], sel)
            due = min(c + 2, nch - 1)
            if c != nch - 3 and due in hid:
                hid[due] = _after(hid[due], sum(done, []), never())
                done = []
        xio[pl.ds(r0, TB), :] = acc.astype(bf16)

        @pl.when(layer == 1)
        def _():
            out_cp(t).start()

    def norm0(i):
        x_cp(i).wait()

        @pl.when(i == 0)
        def _():
            wqv_cp[1].start()

        @pl.when(i == 1)
        def _():
            wk_cp[0].start()
            wo_cp[0].start()
            x_cp(2).start()

        rows = pl.ds(pl.multiple_of(i * TB, TB), TB)
        xn = _ln(xio[rows, :].astype(f32)).astype(bf16)
        xn_ref[rows, :] = xn
        xc_ref[rows, :] = xn

    mz_ref[...] = jnp.zeros(mz_ref.shape, f32)
    loop(L // TB, norm0, "norm0")

    def layer_body(layer):
        loop(2 * NSEG, lambda u: pt_body(layer, u), "pt")

        @pl.when(layer == 0)
        def _():
            w1_cp.wait()
            w2_cp.wait()
            w3_cp.wait()
            w4_cp.wait()

        yc_ref[0:LNC, :] = jnp.zeros((LNC, D), bf16)

        loop(S // TB, lambda t: mix_body(layer, t), "mix")

    loop(2, layer_body, "layer")
    for t in range(S // TB):
        out_cp(t).wait()


@jax.jit
def pallas_interleave_layers__memory_aug_infini_attn__mixer_s_mlp__prompt_kernel(
    A_x: jax.Array,
    A_wq: jax.Array,
    A_wk: jax.Array,
    A_wv: jax.Array,
    A_wo: jax.Array,
    A_beta: jax.Array,
    B_x: jax.Array,
    B_w1: jax.Array,
    B_w2: jax.Array,
    B_w3: jax.Array,
    B_w4: jax.Array,
):
    del B_x
    x = A_x.reshape(S, D)
    beta = A_beta.reshape(1, H)
    any_spec = pl.BlockSpec(memory_space=pl.ANY)
    scratch = [
        pltpu.VMEM((S, D), bf16),
        pltpu.VMEM((4, D, HC), bf16),
        pltpu.VMEM((2, D, HC), bf16),
        pltpu.VMEM((2, GH, 256, D), bf16),
        pltpu.VMEM((2, HC, D), bf16),
        pltpu.VMEM((D, D), bf16),
        pltpu.VMEM((D, D), bf16),
        pltpu.VMEM((D, F), bf16),
        pltpu.VMEM((F, D), bf16),
        pltpu.VMEM((1, H), bf16),
        pltpu.VMEM((S + LNC, D), f32),
        pltpu.VMEM((S + LNC, D), f32),
        pltpu.VMEM((TB + 2 * LNC, D), bf16),
        pltpu.VMEM((S, D), bf16),
        pltpu.VMEM((L, D), bf16),
        pltpu.VMEM((L, D), f32),
        pltpu.VMEM((L, HC), bf16),
        pltpu.VMEM((L, HC), bf16),
        pltpu.VMEM((HC, L), bf16),
        pltpu.VMEM((HC, L), bf16),
        pltpu.VMEM((HC, L), bf16),
        pltpu.VMEM((L, HC), bf16),
        pltpu.VMEM((NG, MZR, 128), f32),
        pltpu.VMEM((MZR, 128), f32),
        pltpu.VMEM((7, 64, 128), f32),
        pltpu.VMEM((2, H // 2, 128), f32),
        pltpu.SMEM((1,), jnp.int32),
        pltpu.SemaphoreType.DMA((14,)),
        pltpu.SemaphoreType.DMA((S // TB,)),
        pltpu.SemaphoreType.DMA((S // TB,)),
    ]
    out = pl.pallas_call(
        _kernel,
        out_shape=jax.ShapeDtypeStruct((S, D), bf16),
        in_specs=[any_spec] * 10,
        out_specs=any_spec,
        scratch_shapes=scratch,
        compiler_params=pltpu.CompilerParams(vmem_limit_bytes=112 * 1024 * 1024),
    )(x, A_wq, A_wk, A_wv, A_wo, beta, B_w1, B_w2, B_w3, B_w4)
    return out.reshape(1, S, D)
```
